```python
import os as _os
_os.environ.setdefault("JAX_PLATFORMS", "cpu")
import jax
import jax.numpy as jnp

def _softmax(x, axis=-1):
    return jax.nn.softmax(x, axis=axis)
def _gelu(x):
    return jax.nn.gelu(x, approximate=True)
def _silu(x):
    return jax.nn.silu(x)
def _sigmoid(x):
    return jax.nn.sigmoid(x)
def _layernorm(x, axis=-1, eps=1e-5):
    m = jnp.mean(x, axis=axis, keepdims=True)
    v = jnp.var(x, axis=axis, keepdims=True)
    return (x - m) / jnp.sqrt(v + eps)
def _scatter_add(tgt, idx, src, axis=0):
    return tgt.at[idx].add(src)
def _segment_sum(src, seg, n):
    return jax.ops.segment_sum(src, seg, n)
class _Rng:
    def __init__(self, key):
        self._k = key
    def _next(self):
        self._k, sub = jax.random.split(self._k)
        return sub
    def normal(self, shape):
        return jax.random.normal(self._next(), shape, dtype=jnp.bfloat16)
    def randint(self, lo, hi, shape):
        return jax.random.randint(self._next(), shape, lo, hi, dtype=jnp.int32)
    def uniform(self, shape, lo=0.0, hi=1.0):
        return jax.random.uniform(self._next(), shape, jnp.bfloat16, lo, hi)
    def permutation(self, n):
        return jax.random.permutation(self._next(), n)


kernel_name = 'gated_mix__grouped_kv_mqa__glu_gated_reglu__prompt'

def setup_inputs():
    _rng = _Rng(jax.random.key(int.from_bytes(__import__("os").urandom(4), "little")))
    _w = (lambda a: (lambda t: t.astype(jnp.bfloat16) if jnp.issubdtype(t.dtype, jnp.floating) else t)(jnp.asarray(a)))
    def _A_setup():
        B, S, D, H = 1, 2048, 1024, 32
        Dh = D // H
        return {
            "x": _w((lambda *s: _rng.normal(s) * 0.05)(B, S, D)),
            "wq": _w((lambda *s: _rng.normal(s) * 0.2)(D, H * Dh)),
            "wk": _w((lambda *s: _rng.normal(s) * 0.2)(D, Dh)),
            "wv": _w((lambda *s: _rng.normal(s) * 0.05)(D, Dh)),
            "wo": _w((lambda *s: _rng.normal(s) * 0.05)(H * Dh, D)),
        }
    _A_in = _A_setup()

    def _B_setup():
        B, S, D, F = 1, 2048, 1024, 3584
        return {
            "x": _w((lambda *s: _rng.normal(s) * 0.05)(B, S, D)),
            "W_gate": _w((lambda *s: _rng.normal(s) * 0.8)(D, F) * (2.0 / D) ** 0.5),
            "W_up": _w((lambda *s: _rng.normal(s) * 0.8)(D, F) * (2.0 / D) ** 0.5),
            "W_down": _w((lambda *s: _rng.normal(s) * 0.8)(F, D) * (1.0 / F) ** 0.5),
        }
    _B_in = _B_setup()

    return {
        "A_x": _A_in["x"],
        "A_wq": _A_in["wq"],
        "A_wk": _A_in["wk"],
        "A_wv": _A_in["wv"],
        "A_wo": _A_in["wo"],
        "B_x": _B_in["x"],
        "B_W_gate": _B_in["W_gate"],
        "B_W_up": _B_in["W_up"],
        "B_W_down": _B_in["W_down"],
        "gate_w": _w((lambda *s: _rng.normal(s) * 0.05)(1024) * 16.0),
    }

def reference(A_x, A_wq, A_wk, A_wv, A_wo, B_x, B_W_gate, B_W_up, B_W_down, gate_w):
    def _A_ref(x, wq, wk, wv, wo):
        B, S, D = x.shape
        H = 32
        Dh = D // H
        q = (lambda x, *d: x.transpose(*d))((x @ wq).reshape(B, S, H, Dh), 0, 2, 1, 3)
        k = x @ wk
        v = x @ wv
        scores = jnp.einsum("bhqd,bkd->bhqk", q, k) * (Dh ** -0.5)
        p = _softmax(scores, axis=-1)
        o = jnp.einsum("bhqk,bkd->bhqd", p, v)
        return (lambda x, *d: x.transpose(*d))(o, 0, 2, 1, 3).reshape(B, S, H * Dh) @ wo

    def _B_ref(x, W_gate, W_up, W_down):
        gate = jnp.einsum("bsd,df->bsf", x, W_gate)
        up = jnp.einsum("bsd,df->bsf", x, W_up)
        gate = gate * (lambda x, dt: x.astype(dt))(gate > 0, gate.dtype)
        h = gate * up
        return jnp.einsum("bsf,fd->bsd", h, W_down)

    x = A_x
    g = _sigmoid((x * gate_w).sum(-1, keepdims=True))
    a = _A_ref(x, A_wq, A_wk, A_wv, A_wo)
    b = _B_ref(x, B_W_gate, B_W_up, B_W_down)
    return g * a + (1 - g) * b
```

```python
import functools
import math

import jax
import jax.numpy as jnp
import jax.experimental.pallas as pl
import jax.experimental.pallas.tpu as pltpu

F32 = jnp.float32
BF16 = jnp.bfloat16
NT = (((1,), (1,)), ((), ()))


def make(TQ=512, CK=128, FC=512, ffn_unroll=False, XCH=8, HU=4, LAG=2, rev=True, NB=4, opaque=True, summode=1, DA=2, DL=1):
    def fn(A_x, A_wq, A_wk, A_wv, A_wo, B_x, B_W_gate, B_W_up, B_W_down, gate_w):
        del B_x
        _, S, D = A_x.shape
        DH = A_wk.shape[1]
        H = D // DH
        F = B_W_gate.shape[1]
        HPG = 128 // DH
        NG = H // HPG
        NQ = S // TQ
        NC = S // CK
        NF = F // FC
        XR = S // XCH
        qscale = (DH ** -0.5) * math.log2(math.e)

        def kernel(x_hbm, wq_hbm, wkt_ref, wvt_ref, wo_hbm, wg_hbm, wu_hbm, wd_hbm, gw_ref,
                   o_ref,
                   x_v, wq_v, wo_v, wg_v, wu_v, wd_v, kpad_v, vt_v, q_v,
                   m0, ot_v, acc_v, z_ref, sems, *sb):
            i = pl.program_id(0)
            s0 = sb[0]

            def x_copy(c):
                return pltpu.make_async_copy(x_hbm.at[pl.ds(c * XR, XR)], x_v.at[pl.ds(c * XR, XR)], sems.at[c])
            w_copies = [
                pltpu.make_async_copy(wq_hbm, wq_v, sems.at[XCH]),
                pltpu.make_async_copy(wo_hbm, wo_v, sems.at[XCH + 1]),
                pltpu.make_async_copy(wg_hbm, wg_v, sems.at[XCH + 2]),
                pltpu.make_async_copy(wu_hbm, wu_v, sems.at[XCH + 3]),
                pltpu.make_async_copy(wd_hbm, wd_v, sems.at[XCH + 4]),
            ]

            def qproj(tile, slot):
                xt = x_v[pl.ds(pl.multiple_of(tile * TQ, TQ), TQ), :]
                q = jnp.dot(xt, wq_v[...], preferred_element_type=F32) * qscale
                q = q.astype(BF16)
                for g in range(NG):
                    q_v[slot * NG + g] = q[:, g * 128:(g + 1) * 128]

            def stage_a_chunk(c, kj, qg, sbuf, mx, z):
                kc = kpad_v[kj, pl.ds(c * CK, CK), :]
                s = jax.lax.dot_general(kc, qg, NT, preferred_element_type=F32)
                sbuf[z, pl.ds(c * CK, CK), :] = s
                for r in range(CK // 8):
                    sr = s[r * 8:(r + 1) * 8, :]
                    mx = sr if mx is None else jnp.maximum(mx, sr)
                return mx

            def stage_b_chunk(c, sbuf, m, acc, l, toks, zv):
                if toks:
                    tk = pltpu.bitcast(toks[0], jnp.int32)
                    for t_ in toks[1:]:
                        tk = tk | pltpu.bitcast(t_, jnp.int32)
                    m = pltpu.bitcast(pltpu.bitcast(m, jnp.int32) | (tk & zv), F32)
                sc = sbuf[0, pl.ds(c * CK, CK), :].reshape(CK // 8, 8, TQ)
                p = jnp.exp2(sc - m[None]).reshape(CK, TQ)
                order = list(range(CK // 8))
                if rev:
                    order = [t * 16 + r for t in range(CK // 128) for r in range(15, -1, -1)]
                if summode == 0:
                    for r in order:
                        pr = p[r * 8:(r + 1) * 8, :]
                        l = pr if l is None else l + pr
                elif summode == 1:
                    ls = None
                    for r in order:
                        pr = p[r * 8:(r + 1) * 8, :]
                        ls = pr if ls is None else ls + pr
                    l = ls if l is None else l + ls
                elif summode == 2:
                    ls = None
                    for r in order[::2]:
                        pr = p[r * 8:(r + 1) * 8, :] + p[(r - 1) * 8:r * 8, :]
                        ls = pr if ls is None else ls + pr
                    l = ls if l is None else l + ls
                elif summode == 3:
                    parts = [p[r * 8:(r + 1) * 8, :] for r in order]
                    while len(parts) > 1:
                        parts = [parts[2 * k] + parts[2 * k + 1] for k in range(len(parts) // 2)]
                    l = parts[0] if l is None else l + parts[0]
                o = jnp.dot(vt_v[:, pl.ds(c * CK, CK)], p.astype(BF16), preferred_element_type=F32)
                return (o if acc is None else acc + o), l

            @pl.when(i == 0)
            def _():
                z_ref[0] = 0
                for c in range(XCH):
                    x_copy(c).start()
                w_copies[0].start()
                wkt = wkt_ref[...]
                wkt4 = jnp.concatenate([wkt] * HPG, axis=0)
                wvt = wvt_ref[...]
                lane = jax.lax.broadcasted_iota(jnp.int32, (XR, 128), 1)
                for c in range(XCH):
                    x_copy(c).wait()
                    xc = x_v[pl.ds(c * XR, XR), :]
                    k4 = jax.lax.dot_general(xc, wkt4, NT, preferred_element_type=F32)
                    for j in range(HPG):
                        kpad_v[j, pl.ds(c * XR, XR), :] = jnp.where(
                            (lane >= j * DH) & (lane < (j + 1) * DH), k4, 0.0).astype(BF16)
                    vt = jax.lax.dot_general(wvt, xc, NT, preferred_element_type=F32)
                    vt_v[:, pl.ds(c * XR, XR)] = vt.astype(BF16)
                for w in w_copies[1:]:
                    w.start()
                w_copies[0].wait()
                qproj(0, 0)
                qg = q_v[0]
                mx = None
                for c in range(NC):
                    mx = stage_a_chunk(c, 0, qg, s0, mx, 0)
                m0[...] = jnp.max(mx, axis=0, keepdims=True)

            slot = i & 1

            @pl.when(i + 1 < NQ)
            def _():
                qproj(i + 1, 1 - slot)

            def head_body(t, carry):
                hb = HU * t
                z = z_ref[0] if opaque else 0
                qgs, kjs = [], []
                for u in range(HU):
                    ha = hb + 1 + u
                    flat = slot * H + ha
                    if u == HU - 1:
                        flat = jnp.where(ha == H, jnp.where(i + 1 < NQ, (1 - slot) * H, slot * H), flat)
                    kjs.append(flat & (HPG - 1))
                    qgs.append(flat >> 2)
                ms = [jnp.broadcast_to(m0[...], (8, TQ))] + [None] * HU
                zv = jnp.full((8, TQ), z_ref[0], jnp.int32)
                mx_hist = {}
                l_hist = {}
                mx = None
                acc = l = None
                qg = None
                for k in range(HU * NC + LAG):
                    if k < HU * NC:
                        u, c = divmod(k, NC)
                        if c == 0:
                            mx = None
                            qg = q_v[qgs[u]]
                        mx = stage_a_chunk(c, kjs[u], qg, sb[(u + 1) % NB], mx, z)
                        mx_hist[k] = mx
                        if c == NC - 1:
                            mfin = jnp.max(mx, axis=0, keepdims=True)
                            ms[u + 1] = jnp.broadcast_to(mfin, (8, TQ))
                    kk = k - LAG
                    if kk >= 0:
                        u, c = divmod(kk, NC)
                        if c == 0:
                            acc = l = None
                        toks = []
                        if DA and (k - DA) in mx_hist:
                            toks.append(mx_hist[k - DA])
                        if DL and (kk - DL) in l_hist:
                            toks.append(l_hist[kk - DL])
                        acc, l = stage_b_chunk(c, sb[u % NB], ms[u], acc, l, toks, zv)
                        l_hist[kk] = l
                        if c == NC - 1:
                            lt = jnp.sum(l, axis=0, keepdims=True)
                            ot_v[pl.ds(pl.multiple_of((hb + u) * DH, DH), DH), :] = acc * (1.0 / lt)
                m0[...] = mfin
                return carry
            jax.lax.fori_loop(0, H // HU, head_body, 0)

            @pl.when(i == 0)
            def _():
                for w in w_copies[1:]:
                    w.wait()

            xt = x_v[pl.ds(pl.multiple_of(i * TQ, TQ), TQ), :]
            gw = gw_ref[...].astype(F32)
            gacc = None
            for r in range(D // 128):
                pr = xt[:, r * 128:(r + 1) * 128].astype(F32) * gw[r:r + 1, :]
                gacc = pr if gacc is None else gacc + pr
            gate = jax.nn.sigmoid(jnp.sum(gacc, axis=1, keepdims=True))
            o_nat = ot_v[...].T.astype(BF16)
            a = jnp.dot(o_nat, wo_v[...], preferred_element_type=F32)
            acc_v[...] = a * gate

            def ffn_body(c, carry):
                off = pl.multiple_of(c * FC, FC) if not isinstance(c, int) else c * FC
                xt = x_v[pl.ds(pl.multiple_of(i * TQ, TQ), TQ), :]
                gg = jnp.dot(xt, wg_v[:, pl.ds(off, FC)], preferred_element_type=F32)
                uu = jnp.dot(xt, wu_v[:, pl.ds(off, FC)], preferred_element_type=F32)
                hh = (jnp.maximum(gg, 0.0) * uu * (1.0 - gate)).astype(BF16)
                acc_v[...] += jnp.dot(hh, wd_v[pl.ds(off, FC), :], preferred_element_type=F32)
                return carry
            if ffn_unroll:
                for c in range(NF):
                    ffn_body(c, 0)
            else:
                jax.lax.fori_loop(0, NF, ffn_body, 0)
            o_ref[...] = acc_v[...].astype(o_ref.dtype)

        any_spec = pl.BlockSpec(memory_space=pl.ANY)
        out = pl.pallas_call(
            kernel,
            grid=(NQ,),
            in_specs=[any_spec, any_spec,
                      pl.BlockSpec((DH, D), lambda i: (0, 0)),
                      pl.BlockSpec((DH, D), lambda i: (0, 0)),
                      any_spec, any_spec, any_spec, any_spec,
                      pl.BlockSpec((D // 128, 128), lambda i: (0, 0))],
            out_specs=pl.BlockSpec((TQ, D), lambda i: (i, 0)),
            out_shape=jax.ShapeDtypeStruct((S, D), A_x.dtype),
            scratch_shapes=[
                pltpu.VMEM((S, D), BF16),
                pltpu.VMEM((D, D), BF16),
                pltpu.VMEM((D, D), BF16),
                pltpu.VMEM((D, F), BF16),
                pltpu.VMEM((D, F), BF16),
                pltpu.VMEM((F, D), BF16),
                pltpu.VMEM((HPG, S, 128), BF16),
                pltpu.VMEM((DH, S), BF16),
                pltpu.VMEM((2 * NG, TQ, 128), BF16),
                pltpu.VMEM((1, TQ), F32),
                pltpu.VMEM((D, TQ), F32),
                pltpu.VMEM((TQ, D), F32),
                pltpu.SMEM((1,), jnp.int32),
                pltpu.SemaphoreType.DMA((XCH + 5,)),
            ] + [pltpu.VMEM((1, S, TQ), F32)] * NB,
            compiler_params=pltpu.CompilerParams(
                dimension_semantics=("arbitrary",),
                vmem_limit_bytes=100 * 1024 * 1024),
            name="gated_mix",
        )(A_x.reshape(S, D), A_wq, A_wk.T, A_wv.T, A_wo, B_W_gate, B_W_up, B_W_down,
          gate_w.reshape(D // 128, 128))
        return out.reshape(1, S, D)
    return jax.jit(fn)


_impl = make(DL=2,LAG=1,opaque=False,ffn_unroll=True)


@jax.jit
def pallas_gated_mix__grouped_kv_mqa__glu_gated_reglu__prompt_kernel(
    A_x: jax.Array,
    A_wq: jax.Array,
    A_wk: jax.Array,
    A_wv: jax.Array,
    A_wo: jax.Array,
    B_x: jax.Array,
    B_W_gate: jax.Array,
    B_W_up: jax.Array,
    B_W_down: jax.Array,
    gate_w: jax.Array,
):
    return _impl(A_x, A_wq, A_wk, A_wv, A_wo, B_x, B_W_gate, B_W_up, B_W_down, gate_w)
```

```python
import math

import jax
import jax.numpy as jnp
import jax.experimental.pallas as pl
import jax.experimental.pallas.tpu as pltpu

F32 = jnp.float32
BF16 = jnp.bfloat16
I32 = jnp.int32
NT = (((1,), (1,)), ((), ()))


def make(TQ=512, CK=128, XCH=8, LAG=1, DA=2, DL=2, NV=192, CW=2, pin_end=True, RH=2, nodma=0, pins=None, PS=0, EVEN=1, WL=1, AOFF=0.0):
    def fn(A_x, A_wq, A_wk, A_wv, A_wo, B_x, B_W_gate, B_W_up, B_W_down, gate_w):
        del B_x
        _, S, D = A_x.shape
        DH = A_wk.shape[1]
        H = D // DH
        F = B_W_gate.shape[1]
        HPG = 128 // DH
        NG = H // HPG
        NQ = S // TQ
        NC = S // CK
        NF = NG // RH
        FC = F // NF
        TR = TQ // RH
        LT = TQ // 128
        XR = S // XCH
        XT0 = TQ // XR
        qscale = (DH ** -0.5) * math.log2(math.e)
        assert NV % 16 == 0 and NV <= XR and XR == TR

        def a_chunks(nv):
            out = []
            if EVEN:
                units = (S - nv) // 16
                lo = nv
                for c in range(NC):
                    n = ((c + 1) * units // NC - c * units // NC) * 16
                    out.append((lo, n))
                    lo += n
                return out
            for c in range(NC):
                lo, hi = max(c * CK, nv), (c + 1) * CK
                if lo < hi:
                    out.append((lo, hi - lo))
            return out

        def kernel(x_hbm, wq_hbm, wkt_hbm, wvt_hbm, wo_hbm, wg_hbm, wu_hbm, wd_hbm, gw_hbm,
                   o_ref,
                   x_v, wq_v, wkt_v, wvt_v, wo_v, wg_v, wu_v, wd_v, gw_v, k_v, vt_v, g_v,
                   kb_v, qta_v, qtb_v, sv0_v, sv_v, m0, ot_v, acc_v, z_ref, sems, sb0, sb1):
            i = pl.program_id(0)
            sb = (sb0, sb1)

            class _Nop:
                def start(self): pass
                def wait(self): pass

            def cp(src, dst, k):
                if nodma == 1 or (nodma == 2 and k >= XCH + 5):
                    return _Nop()
                return pltpu.make_async_copy(src, dst, sems.at[k])

            def x_copy(c):
                return cp(x_hbm.at[pl.ds(c * XR, XR)], x_v.at[pl.ds(c * XR, XR)], c)

            def small_copies():
                return [cp(wkt_hbm, wkt_v, XCH), cp(wvt_hbm, wvt_v, XCH + 1), cp(gw_hbm, gw_v, XCH + 2)]

            def wq_copy(g):
                return cp(wq_hbm.at[:, pl.ds(g * 128, 128)], wq_v.at[g], XCH + 3 + g)

            def wo_copy(part):
                lo, hi = [(0, 128), (128, D)][part]
                sl = pl.ds(lo, hi - lo)
                return cp(wo_hbm.at[sl], wo_v.at[sl], XCH + 3 + NG + part)

            def ffn_copies(f):
                sl = pl.ds(f * FC, FC)
                k = XCH + 5 + NG + 3 * f
                return [cp(wg_hbm.at[:, sl], wg_v.at[f], k),
                        cp(wu_hbm.at[:, sl], wu_v.at[f], k + 1),
                        cp(wd_hbm.at[sl], wd_v.at[f], k + 2)]

            def body_copies(t):
                out = []
                if t == 0:
                    out += [wq_copy(2), wo_copy(0)]
                if t == 1:
                    out += [wq_copy(g) for g in range(3, NG)] + [wo_copy(1)]
                if t % RH == 0:
                    out += ffn_copies(t // RH)
                return out

            def tok_or(x, toks, zv):
                tk = pltpu.bitcast(toks[0], I32)
                for t_ in toks[1:]:
                    tk = tk | pltpu.bitcast(t_, I32)
                return pltpu.bitcast(pltpu.bitcast(x, I32) | (tk & zv), F32)

            def qproj_t(tile, g):
                if isinstance(tile, int):
                    xt = x_v[pl.ds(tile * TQ, TQ), :]
                    w = wq_v[g]
                else:
                    xt = x_v[pl.ds(pl.multiple_of(tile * TQ, TQ), TQ), :]
                    w = wq_v[g]
                q = jnp.dot(xt, w, preferred_element_type=F32) * qscale
                return q.T.astype(BF16)

            def a_chunk(lo, n, qh, dst, mx):
                s = jnp.dot(k_v[pl.ds(lo, n), :], qh, preferred_element_type=F32)
                dst[pl.ds(lo, n), :] = s
                for r in range(n // 8):
                    sr = s[r * 8:(r + 1) * 8, :]
                    mx = sr if mx is None else jnp.maximum(mx, sr)
                return mx

            def b_chunk(c, sc, m, acc, l):
                p = jnp.exp2(sc.reshape(CK // 8, 8, TQ) - m[None]).reshape(CK, TQ)
                ls = None
                for r in range(CK // 8 - 1, -1, -1):
                    pr = p[r * 8:(r + 1) * 8, :]
                    ls = pr if ls is None else ls + pr
                l = ls if l is None else l + ls
                o = jnp.dot(vt_v[:, pl.ds(c * CK, CK)], p.astype(BF16), preferred_element_type=F32)
                return (o if acc is None else acc + o), l

            def vpu_scores(q_ref, row0, prev, zv1, dst):
                rows = []
                mx = None
                for kv in range(NV // 8):
                    parts = []
                    for b0 in range(0, LT, CW):
                        accs = [None] * CW
                        if prev is not None:
                            accs = [pltpu.bitcast(pltpu.bitcast(a, I32) & zv1, F32) for a in prev]
                        for d in range(DH):
                            kk = kb_v[d, kv]
                            for b in range(CW):
                                pr = kk * q_ref[b0 + b, pl.ds(row0 + d, 8, stride=0), :]
                                accs[b] = pr if accs[b] is None else accs[b] + pr
                        prev = accs
                        parts += accs
                        for b in range(CW):
                            dst[kv * 8:(kv + 1) * 8, (b0 + b) * 128:(b0 + b + 1) * 128] = accs[b]
                    row = jnp.concatenate(parts, axis=1)
                    mx = row if mx is None else jnp.maximum(mx, row)
                return dst, mx, prev

            def attention(qhs, svs, mvs, tile, zv, first_tok, full):
                grow = jnp.concatenate([g_v[tile * RH + rr][0:1, :] for rr in range(RH)], axis=1)
                ms = [jnp.broadcast_to(m0[...], (8, TQ))] + [None] * HPG
                ach = a_chunks(0 if full else NV)
                na = len(ach)
                events = []
                for u in range(HPG):
                    for k, _ in enumerate(ach):
                        events.append((u * NC + k * NC / na, 0, "a", u, k))
                    for c in range(NC):
                        events.append((u * NC + c + LAG, 1, "b", u, c))
                events.sort()
                mx_hist, l_hist = [], []
                mx = acc = l = mfin = None
                new_sv0 = None
                for _, _, kind, u, k in events:
                    if kind == "a":
                        lo, n = ach[k]
                        if k == 0:
                            mx = None if full else mvs[u]
                        dst = sb[(u + 1) % 2]
                        if full and u == HPG - 1 and lo < NV:
                            s = jnp.dot(k_v[pl.ds(lo, n), :], qhs[u], preferred_element_type=F32)
                            nn = min(n, NV - lo)
                            new_sv0 = (new_sv0 or []) + [s[:nn]]
                            if nn < n:
                                dst[pl.ds(lo + nn, n - nn), :] = s[nn:]
                            for r in range(n // 8):
                                sr = s[r * 8:(r + 1) * 8, :]
                                mx = sr if mx is None else jnp.maximum(mx, sr)
                        else:
                            mx = a_chunk(lo, n, qhs[u], dst, mx)
                        mx_hist.append(mx)
                        if k == na - 1:
                            mfin = jnp.max(mx, axis=0, keepdims=True)
                            ms[u + 1] = jnp.broadcast_to(mfin, (8, TQ))
                    else:
                        c = k
                        if c == 0:
                            acc = l = None
                        toks = []
                        if DA and len(mx_hist) > DA:
                            toks.append(mx_hist[-1 - DA])
                        if DL and len(l_hist) >= DL:
                            toks.append(l_hist[-DL])
                        if first_tok is not None and u * NC + c == PS:
                            toks.append(first_tok)
                        m = tok_or(ms[u], toks, zv) if toks else ms[u]
                        lo, hi = c * CK, (c + 1) * CK
                        nv = 0 if full else NV
                        pieces = []
                        if lo < nv:
                            e = min(hi, nv)
                            pieces.append(sv0_v[pl.ds(lo, e - lo), :] if u == 0 else svs[u - 1][lo:e, :])
                        if hi > nv:
                            b = max(lo, nv)
                            pieces.append(sb[u % 2][pl.ds(b, hi - b), :])
                        sc = pieces[0] if len(pieces) == 1 else jnp.concatenate(pieces, axis=0)
                        acc, l = b_chunk(c, sc, m, acc, l)
                        l_hist.append(l)
                        if c == NC - 1:
                            lt = jnp.sum(l, axis=0, keepdims=True)
                            on = acc * (grow / lt)
                            for rr in range(RH):
                                ot_v[rr, u * DH:(u + 1) * DH, :] = on[:, rr * TR:(rr + 1) * TR]
                m0[...] = mfin
                sv0_v[...] = jnp.concatenate(new_sv0, axis=0) if full else svs[HPG - 1][...]

            def store_qt(qt, part):
                qf = qt.astype(F32)
                for b in range(LT):
                    if part == "b":
                        qtb_v[b] = qf[0:DH, b * 128:(b + 1) * 128]
                    else:
                        qta_v[b] = qf[DH:, b * 128:(b + 1) * 128]

            def pin_w(w, name, toks, zv1):
                for (nm, rt, ct), tok in toks:
                    if nm != name:
                        continue
                    r0, c0 = rt * 128, ct * 128
                    v = pltpu.bitcast(w[r0:r0 + 16, c0:c0 + 128], I32) | (pltpu.bitcast(tok, I32) & zv1)
                    v = pltpu.bitcast(v, BF16)
                    band = [v]
                    if c0 > 0:
                        band = [w[r0:r0 + 16, :c0]] + band
                    if c0 + 128 < w.shape[1]:
                        band = band + [w[r0:r0 + 16, c0 + 128:]]
                    rows = [jnp.concatenate(band, axis=1)]
                    if r0 > 0:
                        rows = [w[:r0]] + rows
                    if r0 + 16 < w.shape[0]:
                        rows = rows + [w[r0 + 16:]]
                    w = jnp.concatenate(rows, axis=0)
                return w

            def ffn_part(t, toks=(), zv1=None):
                r = t & (RH - 1)
                f = t >> 1
                goff = pl.multiple_of(t * 128, 128)
                wo_g = wo_v[pl.ds(goff, 128), :]
                for rr in range(RH):
                    half = (r + rr) & (RH - 1)
                    row = pl.multiple_of(half * TR, TR)
                    o_nat = ot_v[half].T.astype(BF16)
                    if rr == 0:
                        xt = x_v[pl.ds(pl.multiple_of(i * TQ + row, TR), TR), :]
                        gb = jnp.broadcast_to(1.0 - g_v[i * RH + half][0:1, :], (128, TR)).T
                        gg = jnp.dot(xt, pin_w(wg_v[f], 'g', toks, zv1), preferred_element_type=F32)
                        uu = jnp.dot(xt, pin_w(wu_v[f], 'u', toks, zv1), preferred_element_type=F32)
                        hh = jnp.maximum(gg, 0.0) * uu
                        hh = jnp.concatenate(
                            [hh[:, j * 128:(j + 1) * 128] * gb for j in range(FC // 128)],
                            axis=1).astype(BF16)
                        y = jnp.dot(o_nat, wo_g, preferred_element_type=F32)
                        y = y + jnp.dot(hh, pin_w(wd_v[f], 'd', toks, zv1), preferred_element_type=F32)
                    else:
                        y = jnp.dot(o_nat, pin_w(wo_g, 'o', toks, zv1), preferred_element_type=F32)
                    y = y + jnp.where(t > 0, acc_v[pl.ds(row, TR), :], 0.0)
                    acc_v[pl.ds(row, TR), :] = y
                    o_ref[pl.ds(row, TR), :] = y.astype(o_ref.dtype)

            @pl.when(i == 0)
            def _():
                z_ref[0] = 0
                for c_ in small_copies():
                    c_.start()
                for c in range(XT0):
                    x_copy(c).start()
                wq_copy(0).start()
                wq_copy(1).start()
                for c in range(XT0, XCH):
                    x_copy(c).start()
                for t in range(NG):
                    for c_ in body_copies(t):
                        c_.start()
                for c_ in small_copies():
                    c_.wait()
                gw = gw_v[...].astype(F32)
                gw_row = jnp.concatenate([gw[r:r + 1, :] for r in range(D // 128)], axis=1)
                gw16 = jnp.broadcast_to(gw_row, (16, D)).astype(BF16)
                wvg = jnp.concatenate([wvt_v[...], gw16], axis=0)
                mx = None
                qt0 = qt1 = None
                cdone = 0
                for c in range(XCH):
                    x_copy(c).wait()
                    xc = x_v[pl.ds(c * XR, XR), :]
                    k1 = jax.lax.dot_general(xc, wkt_v[...], NT, preferred_element_type=F32).astype(BF16)
                    k_v[pl.ds(c * XR, XR), :] = k1
                    if c == 0:
                        kf = k1[:NV].astype(F32)
                        for d in range(DH):
                            kb_v[d] = jnp.broadcast_to(kf[:, d:d + 1], (NV, 128)).reshape(NV // 8, 8, 128)
                    vt = jax.lax.dot_general(wvg, xc, NT, preferred_element_type=F32)
                    vt_v[:, pl.ds(c * XR, XR)] = vt[:DH].astype(BF16)
                    g_v[c] = jax.nn.sigmoid(vt[DH:DH + 8])
                    if c == XT0 - 1:
                        wq_copy(0).wait()
                        qt0 = qproj_t(0, 0)
                    if c == XT0:
                        wq_copy(1).wait()
                        qt1 = qproj_t(0, 1)
                        store_qt(qt1, "a")
                    if qt0 is not None:
                        while (cdone + 1) * CK <= (c + 1) * XR:
                            mx = a_chunk(cdone * CK, CK, qt0[0:DH], sb[0], mx)
                            cdone += 1
                m0[...] = jnp.max(mx, axis=0, keepdims=True)
                zv = jnp.full((8, TQ), z_ref[0], I32)
                qhs = [qt0[DH * j:DH * (j + 1)] for j in range(1, HPG)] + [qt1[0:DH]]
                attention(qhs, None, None, 0, zv, None, True)

            def body(t, carry):
                def waits(_, c0):
                    for tt in range(NG):
                        if tt <= 1 or tt % RH == 0:
                            @pl.when(t == tt)
                            def _():
                                for c_ in body_copies(tt):
                                    c_.wait()
                    return c0
                if WL:
                    jax.lax.fori_loop(0, jnp.where(i == 0, 1, 0), waits, 0)
                else:
                    pl.when(i == 0)(lambda: waits(0, None))

                zv = jnp.full((8, TQ), z_ref[0], I32)
                zv1 = zv[:, :128]
                it = i * NG + t
                g2 = jnp.minimum(it + 2, NQ * NG - 1)
                qt_new = qproj_t(g2 >> 3, g2 & (NG - 1))
                store_qt(qt_new, "b")
                svs, mvs, ends = [], [], []
                prev = None
                for j in range(1, HPG):
                    sv, mv, prev = vpu_scores(qta_v, (j - 1) * DH, prev, zv1, sv_v.at[j - 1])
                    svs.append(sv)
                    mvs.append(mv)
                    ends.append(prev[0])
                sv, mv, prev = vpu_scores(qtb_v, 0, prev, zv1, sv_v.at[HPG - 1])
                svs.append(sv)
                mvs.append(mv)
                ends.append(prev[0])
                ffn_part(t, [(p_, e_) for p_, e_ in zip(pins or [], ends) if p_ is not None], zv1)
                qa = jnp.concatenate([qta_v[b] for b in range(LT)], axis=1).astype(BF16)
                qhs = [qa[DH * j:DH * (j + 1)] for j in range(HPG - 1)] + [qt_new[0:DH]]
                attention(qhs, svs, mvs, (it + 1) >> 3, zv, mv if pin_end else None, False)
                store_qt(qt_new, "a")
                return carry
            jax.lax.fori_loop(0, jnp.where(i == NQ - 1, NG - 1, NG), body, 0)

            @pl.when(i == NQ - 1)
            def _():
                ffn_part(jnp.int32(NG - 1))

        any_spec = pl.BlockSpec(memory_space=pl.ANY)
        out = pl.pallas_call(
            kernel,
            grid=(NQ,),
            in_specs=[any_spec] * 9,
            out_specs=pl.BlockSpec((TQ, D), lambda i: (i, 0)),
            out_shape=jax.ShapeDtypeStruct((S, D), A_x.dtype),
            scratch_shapes=[
                pltpu.VMEM((S, D), BF16),
                pltpu.VMEM((NG, D, 128), BF16),
                pltpu.VMEM((DH, D), BF16),
                pltpu.VMEM((DH, D), BF16),
                pltpu.VMEM((D, D), BF16),
                pltpu.VMEM((NF, D, FC), BF16),
                pltpu.VMEM((NF, D, FC), BF16),
                pltpu.VMEM((NF, FC, D), BF16),
                pltpu.VMEM((D // 128, 128), BF16),
                pltpu.VMEM((S, DH), BF16),
                pltpu.VMEM((DH, S), BF16),
                pltpu.VMEM((XCH, 8, XR), F32),
                pltpu.VMEM((DH, NV // 8, 8, 128), F32),
                pltpu.VMEM((LT, 128 - DH, 128), F32),
                pltpu.VMEM((LT, DH, 128), F32),
                pltpu.VMEM((NV, TQ), F32),
                pltpu.VMEM((HPG, NV, TQ), F32),
                pltpu.VMEM((1, TQ), F32),
                pltpu.VMEM((RH, 128, TR), F32),
                pltpu.VMEM((TQ, D), F32),
                pltpu.SMEM((1,), I32),
                pltpu.SemaphoreType.DMA((XCH + 5 + NG + 3 * NF,)),
                pltpu.VMEM((S, TQ), F32),
                pltpu.VMEM((S, TQ), F32),
            ],
            compiler_params=pltpu.CompilerParams(
                dimension_semantics=("arbitrary",),
                vmem_limit_bytes=100 * 1024 * 1024),
            name="gated_mix",
        )(A_x.reshape(S, D), A_wq, A_wk.T, A_wv.T, A_wo, B_W_gate, B_W_up, B_W_down,
          gate_w.reshape(D // 128, 128))
        return out.reshape(1, S, D)
    return jax.jit(fn)


_impl = make(NV=160,PS=2,LAG=0)


@jax.jit
def pallas_gated_mix__grouped_kv_mqa__glu_gated_reglu__prompt_kernel(
    A_x: jax.Array,
    A_wq: jax.Array,
    A_wk: jax.Array,
    A_wv: jax.Array,
    A_wo: jax.Array,
    B_x: jax.Array,
    B_W_gate: jax.Array,
    B_W_up: jax.Array,
    B_W_down: jax.Array,
    gate_w: jax.Array,
):
    return _impl(A_x, A_wq, A_wk, A_wv, A_wo, B_x, B_W_gate, B_W_up, B_W_down, gate_w)
```

```python
import math

import jax
import jax.numpy as jnp
import jax.experimental.pallas as pl
import jax.experimental.pallas.tpu as pltpu

F32 = jnp.float32
BF16 = jnp.bfloat16
I32 = jnp.int32
NT = (((1,), (1,)), ((), ()))


TQ = 512
TR = 256
CK = 128
NV = 256
LAG = 2
TA = 3
NEXT0 = 40
ESPLIT = 4


@jax.jit
def pallas_gated_mix__grouped_kv_mqa__glu_gated_reglu__prompt_kernel(
    A_x: jax.Array,
    A_wq: jax.Array,
    A_wk: jax.Array,
    A_wv: jax.Array,
    A_wo: jax.Array,
    B_x: jax.Array,
    B_W_gate: jax.Array,
    B_W_up: jax.Array,
    B_W_down: jax.Array,
    gate_w: jax.Array,
):
    del B_x
    _, S, D = A_x.shape
    DH = A_wk.shape[1]
    F = B_W_gate.shape[1]
    HPG = 128 // DH
    NG = D // 128
    NQ = S // TQ
    NIT = NQ * NG
    NC = S // CK
    RH = TQ // TR
    NF = NG // RH
    FC = F // NF
    LT = TQ // 128
    XCH = S // TR
    KA = DH + 16
    qscale = (DH ** -0.5) * math.log2(math.e)
    assert NG == 8 and RH == 2 and LT == 4 and HPG == 4 and FC % 128 == 0
    assert NV % 16 == 0 and NV <= TQ
    ngr = NV // 16
    nvg = [(c + 1) * ngr // NC - c * ngr // NC for c in range(NC)]
    vk = [(sum(nvg[:c]) * 16, nvg[c] * 16) for c in range(NC)]
    mk = [(NV + c * CK - vk[c][0], CK - vk[c][1]) for c in range(NC)]

    SEM_SMALL = XCH
    SEM_WQ = XCH + 1
    SEM_BODY = XCH + 4
    BODY_SEM = {t: SEM_BODY + n
                for n, t in enumerate(t for t in range(NG) if t <= 1 or t % RH == 0)}
    NSEM = SEM_BODY + len(BODY_SEM)
    SEM_OUT = 0

    def kernel(x_hbm, wq_hbm, wkt_hbm, wvt_hbm, wo_hbm, wg_hbm, wu_hbm, wd_hbm, gw_hbm,
               o_hbm,
               x_v, wq_v, wkt_v, wvt_v, wo_v, wg_v, wu_v, wd_v, gw_v, wkv_v,
               k_v, ka_v, vt_v, vn_v, vp_v, g_v, vb_v,
               kb_v, qa_v, sh0_v, qs_v, p0_v, sv_v, l0_v, ot_v, acc_v, o_v, sf_v, z_ref, sems):

        def cp(src, dst, k):
            return pltpu.make_async_copy(src, dst, sems.at[k])

        def al(v, m):
            return v if isinstance(v, int) else pl.multiple_of(v, m)

        def x_copy(c):
            rows = pl.ds(al(c * TR, TR), TR)
            return cp(x_hbm.at[rows], x_v.at[rows], c)

        def small_copies():
            return [cp(wkt_hbm, wkt_v, SEM_SMALL), cp(wvt_hbm, wvt_v, SEM_SMALL),
                    cp(gw_hbm, gw_v, SEM_SMALL)]

        def wq_copy(g):
            k = SEM_WQ + g if g < 3 else BODY_SEM[min(g - 3, 1)]
            return cp(wq_hbm.at[:, pl.ds(g * 128, 128)], wq_v.at[g], k)

        def wo_copy(part):
            lo, hi = [(0, 128), (128, D)][part]
            sl = pl.ds(lo, hi - lo)
            return cp(wo_hbm.at[sl], wo_v.at[sl], BODY_SEM[part])

        def body_copies(t):
            out = []
            if t == 0:
                out += [wq_copy(3), wo_copy(0)]
            if t == 1:
                out += [wq_copy(g) for g in range(4, NG)] + [wo_copy(1)]
            if t % RH == 0:
                f = t // RH
                sl = pl.ds(f * FC, FC)
                out += [cp(wg_hbm.at[:, sl], wg_v.at[f], BODY_SEM[t]),
                        cp(wu_hbm.at[:, sl], wu_v.at[f], BODY_SEM[t]),
                        cp(wd_hbm.at[sl], wd_v.at[f], BODY_SEM[t])]
            return out

        def out_copy(tile, lo=0, n=TQ, k=None):
            k = SEM_OUT + tile % 2 if k is None else k
            return cp(o_v.at[tile % 2, pl.ds(lo, n)], o_hbm.at[pl.ds(tile * TQ + lo, n)], k)

        def tie(x, tok, zv):
            bits = pltpu.bitcast(x, I32) | (pltpu.bitcast(tok, I32) & zv)
            return pltpu.bitcast(bits, x.dtype)

        def fold(op, s, r0=None):
            for r in range(s.shape[0] // 8):
                sr = s[r * 8:(r + 1) * 8, :]
                r0 = sr if r0 is None else op(r0, sr)
            return r0

        def qproj_t(tile, g):
            xt = x_v[pl.ds(al(tile * TQ, TQ), TQ), :]
            q = jnp.dot(xt, wq_v[g], preferred_element_type=F32) * qscale
            return q.T.astype(BF16)

        def store_q(qt, row0):
            qf = qt.astype(F32)
            for b in range(LT):
                qa_v[b, row0:row0 + 128, :] = qf[:, b * 128:(b + 1) * 128]

        def vpu_chain(zv1):
            mrows = []
            prev = None
            for j in range(HPG):
                row0 = (j + 1) * DH
                mx = None
                for kv in range(NV // 8):
                    parts = []
                    for b0 in range(0, LT, 2):
                        accs = [None, None]
                        if prev is not None:
                            tks = [pltpu.bitcast(a, I32) for a in prev]
                            if mx is not None:
                                tks = [tk | pltpu.bitcast(mx[:, (b0 + b) * 128:(b0 + b + 1) * 128], I32)
                                       for b, tk in enumerate(tks)]
                            accs = [pltpu.bitcast(tk & zv1, F32) for tk in tks]
                        for d in range(DH):
                            kk = kb_v[d, kv]
                            for b in range(2):
                                pr = kk * qa_v[b0 + b, pl.ds(row0 + d, 8, stride=0), :]
                                accs[b] = pr if accs[b] is None else accs[b] + pr
                        prev = accs
                        parts += accs
                        for b in range(2):
                            sv_v[j, kv * 8:(kv + 1) * 8, (b0 + b) * 128:(b0 + b + 1) * 128] = accs[b]
                    row = jnp.concatenate(parts, axis=1)
                    mx = row if mx is None else jnp.maximum(mx, row)
                mrows.append(jnp.max(mx, axis=0, keepdims=True))
            return mrows

        def gate_row(tile):
            return jnp.concatenate([g_v[tile * RH + rr][0:1, :] for rr in range(RH)], axis=1)

        def put_ot(u, on):
            for rr in range(RH):
                ot_v[rr, pl.ds(al(u * DH, DH), DH), :] = on[:, rr * TR:(rr + 1) * TR]

        def shift_of(mrow):
            sub = jax.lax.broadcasted_iota(I32, (16, TQ), 0)
            hi = mrow.astype(BF16).astype(F32)
            lo = (mrow - hi).astype(BF16).astype(F32)
            shift = jnp.where(sub == 0, -hi, jnp.where(sub == 1, -lo, 0.0)).astype(BF16)
            return shift, jnp.broadcast_to(hi + lo, (8, TQ))

        def attention(qt, mrows, tile, zv, tail_fn=None):
            grow = gate_row(tile)
            events = []
            for u in range(HPG):
                for c in range(NC):
                    events.append((u * NC + c, 1, "qk", u, c))
                    events.append((u * NC + c + LAG, 0, "pv", u, c))
            if tail_fn is not None:
                events.append((HPG * NC, 0.5, "tail", 0, 0))
                for g_ in range(NV // 16):
                    events.append((NEXT0 + g_, 0.6, "next", 0, g_))
            events.sort()
            s_val, st, nxt = {}, {}, {}
            l_hist, a_hist = [], []
            bad = None
            for _, _, kind, u, c in events:
                if kind == "tail":
                    tail_fn()
                    continue
                if kind == "next":
                    if not nxt:
                        nxt["shift"], nxt["m"] = shift_of(mrows[HPG])
                        nxt["l"] = None
                    m = tie(nxt["m"], l_hist[-2], zv)
                    p = jnp.exp2(sv_v[HPG - 1, c * 16:(c + 1) * 16, :].reshape(2, 8, TQ) - m[None])
                    p = p.reshape(16, TQ)
                    nxt["l"] = fold(jnp.add, p, nxt["l"])
                    p0_v[c * 16:(c + 1) * 16, :] = p
                    if c == NV // 16 - 1:
                        sh0_v[...] = nxt["shift"]
                        l0_v[...] = nxt["l"]
                    continue
                if u not in st:
                    pre = mrows[u] is None
                    shift, mb = (sh0_v[...], l0_v[...]) if pre else shift_of(mrows[u])
                    st[u] = dict(q=qt[u * DH:(u + 1) * DH], shift=shift, m=mb, acc=None,
                                 l=mb if pre else None, pre=pre)
                h = st[u]
                if kind == "qk":
                    k_ = u * NC + c
                    sh = tie(h["shift"], a_hist[k_ - TA], zv) if k_ >= TA else h["shift"]
                    w = jnp.concatenate([h["q"], sh], axis=0)
                    s_val[(u, c)] = jnp.dot(ka_v[pl.ds(*mk[c]), :], w, preferred_element_type=F32)
                    continue
                pv = None
                if vk[c][1]:
                    sc = (p0_v if u == 0 else sv_v.at[u - 1])[pl.ds(*vk[c]), :]
                    if h["pre"]:
                        pv = sc
                    else:
                        pv = jnp.exp2(sc.reshape(vk[c][1] // 8, 8, TQ) - h["m"][None])
                        pv = pv.reshape(vk[c][1], TQ)
                pm = jnp.exp2(s_val.pop((u, c)))
                ls = fold(jnp.add, pm)
                if pv is not None and not h["pre"]:
                    ls = fold(jnp.add, pv, ls)
                groups = [pm[j * 16:(j + 1) * 16] for j in range(mk[c][1] // 16 - 1, -1, -1)]
                if pv is not None:
                    groups = [pv] + groups
                p = jnp.concatenate(groups, axis=0).astype(BF16)
                o = jnp.dot(vp_v[:, pl.ds(c * CK, CK)], p, preferred_element_type=F32)
                h["acc"] = o if h["acc"] is None else h["acc"] + o
                h["l"] = ls if h["l"] is None else h["l"] + ls
                l_hist.append(h["l"])
                a_hist.append(h["acc"][DH - 8:, :])
                if c == NC - 1:
                    lt = jnp.sum(h["l"], axis=0, keepdims=True)
                    put_ot(u, h["acc"] * (grow / lt))
                    ok = jnp.logical_and(lt < 2.0 ** 64, lt > 2.0 ** -64)
                    b_ = jnp.where(ok, 0.0, 1.0)
                    bad = b_ if bad is None else jnp.maximum(bad, b_)
            qs_v[...] = qt
            z_ref[1] = jnp.max(bad).astype(I32) | z_ref[2]

        def exact_attention(tile):
            grow = gate_row(tile)

            def head(u, carry):
                w = qs_v[pl.ds(al(u * DH, DH), DH), :]

                def p1(c, mx):
                    rows = pl.ds(al(c * CK, CK), CK)
                    s = jnp.dot(k_v[rows, :], w, preferred_element_type=F32)
                    sf_v[rows, :] = s
                    return fold(jnp.maximum, s, mx)
                mx = jax.lax.fori_loop(0, NC, p1, jnp.full((8, TQ), -jnp.inf, F32))
                m = jnp.max(mx, axis=0, keepdims=True)

                def p2(c, carry2):
                    acc, l = carry2
                    rows = pl.ds(al(c * CK, CK), CK)
                    p = jnp.exp2(sf_v[rows, :] - m)
                    o = jnp.dot(vt_v[:, rows], p.astype(BF16), preferred_element_type=F32)
                    return acc + o, fold(jnp.add, p, l)
                acc, l = jax.lax.fori_loop(
                    0, NC, p2, (jnp.zeros((DH, TQ), F32), jnp.zeros((8, TQ), F32)))
                put_ot(u, acc * (grow / jnp.sum(l, axis=0, keepdims=True)))
                return carry
            jax.lax.fori_loop(0, HPG, head, 0)

        def fix_up(tile):
            @pl.when(z_ref[1] != 0)
            def _():
                exact_attention(tile)

        def hidden(tile, half, f):
            xt = x_v[pl.ds(al(tile * TQ + half * TR, TR), TR), :]
            gb = jnp.broadcast_to(1.0 - g_v[tile * RH + half][0:1, :], (128, TR)).T
            gg = jnp.dot(xt, wg_v[f], preferred_element_type=F32)
            uu = jnp.dot(xt, wu_v[f], preferred_element_type=F32)
            hh = jnp.maximum(gg, 0.0) * uu
            return jnp.concatenate(
                [hh[:, j * 128:(j + 1) * 128] * gb for j in range(FC // 128)], axis=1).astype(BF16)

        def ffn_part(tile, t):
            f = t >> 1
            wo_g = wo_v[pl.ds(al(t * 128, 128), 128), :]

            def old(row):
                return jnp.where(t > 0, acc_v[pl.ds(row, TR), :], 0.0)

            half = t & 1
            row = al(half * TR, TR)
            o_nat = ot_v[half].T.astype(BF16)
            hh = hidden(tile, half, f)
            y = jnp.dot(o_nat, wo_g, preferred_element_type=F32)
            y = y + jnp.dot(hh, wd_v[f], preferred_element_type=F32)
            y = y + old(row)
            acc_v[pl.ds(row, TR), :] = y
            o_v[tile & 1, pl.ds(row, TR), :] = y.astype(o_v.dtype)

            half1 = (t + 1) & 1
            row1 = al(half1 * TR, TR)
            o_nat1 = ot_v[half1].T.astype(BF16)

            def tail():
                y1 = jnp.dot(o_nat1, wo_g, preferred_element_type=F32)
                acc_v[pl.ds(row1, TR), :] = y1 + old(row1)
            return tail

        z_ref[0] = 0
        z_ref[1] = 0
        for c_ in small_copies():
            c_.start()
        for c in range(RH):
            x_copy(c).start()
        wq_copy(0).start()
        wq_copy(1).start()
        for c in range(RH, XCH):
            x_copy(c).start()
        wq_copy(2).start()
        for t in range(NG):
            for c_ in body_copies(t):
                c_.start()
        for b in range(LT):
            qa_v[b, 256:, :] = jnp.zeros((8, 128), F32)
        for c_ in small_copies():
            c_.wait()
        gw = gw_v[...].astype(F32)
        gw_row = jnp.concatenate([gw[r:r + 1, :] for r in range(D // 128)], axis=1)
        gw16 = jnp.broadcast_to(gw_row, (16, D)).astype(BF16)
        wkv_v[...] = jnp.concatenate([wvt_v[...], gw16, wkt_v[...]], axis=0)

        def kv_chunk(c):
            rows = pl.ds(al(c * TR, TR), TR)
            vt = jax.lax.dot_general(wkv_v[...], x_v[rows, :], NT, preferred_element_type=F32)
            ones = jnp.where(jax.lax.broadcasted_iota(I32, (16, TR), 0) < 2, 1.0, 0.0)
            ka = jnp.concatenate([vt[DH + 16:], ones], axis=0).T
            k_v[rows, :] = ka[:, 0:DH].astype(BF16)
            ka_v[rows, :] = ka.astype(BF16)
            vn_v[rows, :] = vt[:DH].T
            vt_v[:, rows] = vt[:DH].astype(BF16)
            g_v[c] = jax.nn.sigmoid(vt[DH:DH + 8])
            vb_v[c] = jnp.where(fold(jnp.maximum, jnp.abs(vt[:DH])) < 2.0 ** 60, 0.0, 1.0)

        def kb_rows(ds_):
            kf = k_v[0:NV, :].astype(F32)
            for d in ds_:
                kb_v[d] = jnp.broadcast_to(kf[:, d:d + 1], (NV, 128)).reshape(NV // 8, 8, 128)

        def head_start(qh, dst):
            s = jnp.dot(k_v[0:NV, :], qh, preferred_element_type=F32)
            dst[...] = s
            return jnp.max(fold(jnp.maximum, s), axis=0, keepdims=True)

        for c in range(RH):
            x_copy(c).wait()
            kv_chunk(c)
        wq_copy(0).wait()
        qt0 = qproj_t(0, 0)
        mrows = [head_start(qt0[0:DH], p0_v)]
        mrows += [head_start(qt0[j * DH:(j + 1) * DH], sv_v.at[j - 1]) for j in range(1, HPG)]
        kb_rows(range(0, DH // 2))
        x_copy(RH).wait()
        kv_chunk(RH)
        wq_copy(1).wait()
        qt1 = qproj_t(0, 1)
        m_new = head_start(qt1[0:DH], sv_v.at[HPG - 1])
        store_q(qt1, 0)
        kb_rows(range(DH // 2, DH))

        def xbody(cc, carry):
            x_copy(cc).wait()
            kv_chunk(cc)
            return carry
        jax.lax.fori_loop(RH + 1, XCH - 1, xbody, 0)
        x_copy(XCH - 1).wait()
        wq_copy(2).wait()
        kv_chunk(XCH - 1)
        store_q(qproj_t(0, 2), 128)
        for c in range(NC):
            rows_ = [vn_v[pl.ds(mk[c][0] + j * 16, 16), :] for j in range(mk[c][1] // 16 - 1, -1, -1)]
            if vk[c][1]:
                rows_ = [vn_v[pl.ds(*vk[c]), :]] + rows_
            vp_v[:, pl.ds(c * CK, CK)] = jnp.concatenate(rows_, axis=0).T.astype(BF16)
        z_ref[2] = jnp.max(vb_v[...]).astype(I32)
        attention(qt0, mrows, 0, jnp.full((8, TQ), z_ref[0], I32))
        shift, m = shift_of(m_new)
        sh0_v[...] = shift
        p = jnp.exp2(sv_v[HPG - 1].reshape(NV // 8, 8, TQ) - m[None]).reshape(NV, TQ)
        l0_v[...] = fold(jnp.add, p)
        p0_v[...] = p

        def body(it, carry):
            tile = it >> 3
            t = it & (NG - 1)

            def rare(_, c0):
                for tt in BODY_SEM:
                    @pl.when(it == tt)
                    def _():
                        for c_ in body_copies(tt):
                            c_.wait()
                for q in range(1, NQ):
                    @pl.when(it == q * NG)
                    def _():
                        if q >= 2:
                            out_copy(q - 2).wait()
                        o_v[(q - 1) % 2, 0:TR, :] = acc_v[0:TR, :].astype(o_v.dtype)
                        out_copy(q - 1).start()
                fix_up(tile)
                return c0
            is_rare = jnp.logical_or(jnp.logical_or(it < NG, t == 0), z_ref[1] != 0)
            jax.lax.fori_loop(0, jnp.where(is_rare, 1, 0), rare, 0)

            zv = jnp.full((8, TQ), z_ref[0], I32)
            g3 = jnp.minimum(it + 3, NIT - 1)
            qt_new = qproj_t(g3 >> 3, g3 & (NG - 1))
            mrows = [None] + vpu_chain(zv[:, :128])
            tail_fn = ffn_part(tile, t)
            qt = jnp.concatenate([qa_v[b, 0:128, :] for b in range(LT)], axis=1).astype(BF16)
            attention(qt, mrows, (it + 1) >> 3, zv, tail_fn)
            for b in range(LT):
                qa_v[b, 0:128, :] = qa_v[b, 128:256, :]
            store_q(qt_new, 128)
            return carry
        jax.lax.fori_loop(0, NIT - 1, body, 0)
        fix_up(NQ - 1)

        tile, t = NQ - 1, NG - 1
        half = t % RH
        other = 1 - half
        wo_g = wo_v[t * 128:(t + 1) * 128, :]
        hh = hidden(tile, half, t // RH)
        y = jnp.dot(ot_v[other].T.astype(BF16), wo_g, preferred_element_type=F32)
        y = y + acc_v[other * TR:(other + 1) * TR, :]
        o_v[tile % 2, other * TR:(other + 1) * TR, :] = y.astype(o_v.dtype)
        tail = [out_copy(tile, other * TR, TR, SEM_OUT + 2 + ESPLIT)]
        o_nat = ot_v[half].T.astype(BF16)
        tail[0].start()
        ER = TR // ESPLIT
        for e in range(ESPLIT):
            lo = half * TR + e * ER
            y = jnp.dot(o_nat[e * ER:(e + 1) * ER], wo_g, preferred_element_type=F32)
            y = y + jnp.dot(hh[e * ER:(e + 1) * ER], wd_v[t // RH], preferred_element_type=F32)
            y = y + acc_v[lo:lo + ER, :]
            o_v[tile % 2, lo:lo + ER, :] = y.astype(o_v.dtype)
            tail.append(out_copy(tile, lo, ER, SEM_OUT + 2 + e))
            tail[-1].start()
        out_copy(NQ - 2).wait()
        for c_ in tail:
            c_.wait()

    any_spec = pl.BlockSpec(memory_space=pl.ANY)
    out = pl.pallas_call(
        kernel,
        in_specs=[any_spec] * 9,
        out_specs=any_spec,
        out_shape=jax.ShapeDtypeStruct((S, D), A_x.dtype),
        scratch_shapes=[
            pltpu.VMEM((S, D), BF16),
            pltpu.VMEM((NG, D, 128), BF16),
            pltpu.VMEM((DH, D), BF16),
            pltpu.VMEM((DH, D), BF16),
            pltpu.VMEM((D, D), BF16),
            pltpu.VMEM((NF, D, FC), BF16),
            pltpu.VMEM((NF, D, FC), BF16),
            pltpu.VMEM((NF, FC, D), BF16),
            pltpu.VMEM((D // 128, 128), BF16),
            pltpu.VMEM((2 * DH + 16, D), BF16),
            pltpu.VMEM((S, DH), BF16),
            pltpu.VMEM((S, KA), BF16),
            pltpu.VMEM((DH, S), BF16),
            pltpu.VMEM((S, DH), F32),
            pltpu.VMEM((DH, S), BF16),
            pltpu.VMEM((XCH, 8, TR), F32),
            pltpu.VMEM((XCH, 8, TR), F32),
            pltpu.VMEM((DH, NV // 8, 8, 128), F32),
            pltpu.VMEM((LT, 256 + 8, 128), F32),
            pltpu.VMEM((16, TQ), BF16),
            pltpu.VMEM((128, TQ), BF16),
            pltpu.VMEM((NV, TQ), F32),
            pltpu.VMEM((HPG, NV, TQ), F32),
            pltpu.VMEM((8, TQ), F32),
            pltpu.VMEM((RH, 128, TR), F32),
            pltpu.VMEM((TQ, D), F32),
            pltpu.VMEM((2, TQ, D), A_x.dtype),
            pltpu.VMEM((S, TQ), F32),
            pltpu.SMEM((3,), I32),
            pltpu.SemaphoreType.DMA((NSEM,)),
        ],
        compiler_params=pltpu.CompilerParams(vmem_limit_bytes=100 * 1024 * 1024),
        name="gated_mix",
    )(A_x.reshape(S, D), A_wq, A_wk.T, A_wv.T, A_wo, B_W_gate, B_W_up, B_W_down,
      gate_w.reshape(D // 128, 128))
    return out.reshape(1, S, D)
```

```python
import math

import jax
import jax.numpy as jnp
import jax.experimental.pallas as pl
import jax.experimental.pallas.tpu as pltpu

F32 = jnp.float32
BF16 = jnp.bfloat16
I32 = jnp.int32
NT = (((1,), (1,)), ((), ()))


TQ = 512
TR = 256
CK = 128
NV = 256
LAG = 2
TA = 3
ESPLIT = 4
NEXT0 = 40
QA0, QA_STEP = 24, 0.7
QB0, QB_STEP = 42, 0.8


@jax.jit
def pallas_gated_mix__grouped_kv_mqa__glu_gated_reglu__prompt_kernel(
    A_x: jax.Array,
    A_wq: jax.Array,
    A_wk: jax.Array,
    A_wv: jax.Array,
    A_wo: jax.Array,
    B_x: jax.Array,
    B_W_gate: jax.Array,
    B_W_up: jax.Array,
    B_W_down: jax.Array,
    gate_w: jax.Array,
):
    del B_x
    _, S, D = A_x.shape
    DH = A_wk.shape[1]
    F = B_W_gate.shape[1]
    HPG = 128 // DH
    NG = D // 128
    NQ = S // TQ
    NIT = NQ * NG
    NC = S // CK
    RH = TQ // TR
    NF = NG // RH
    FC = F // NF
    LT = TQ // 128
    XCH = S // TR
    KA = DH + 16
    qscale = (DH ** -0.5) * math.log2(math.e)
    assert NG == 8 and RH == 2 and LT == 4 and HPG == 4 and FC % 128 == 0
    assert NV % 16 == 0 and NV <= TQ
    ngr = NV // 16
    nvg = [(c + 1) * ngr // NC - c * ngr // NC for c in range(NC)]
    vk = [(sum(nvg[:c]) * 16, nvg[c] * 16) for c in range(NC)]
    mk = [(NV + c * CK - vk[c][0], CK - vk[c][1]) for c in range(NC)]

    SEM_SMALL = XCH
    SEM_WQ = XCH + 1
    SEM_BODY = XCH + 4
    BODY_SEM = {t: SEM_BODY + n
                for n, t in enumerate(t for t in range(NG) if t <= 1 or t % RH == 0)}
    NSEM = SEM_BODY + len(BODY_SEM)
    SEM_OUT = 0

    def kernel(x_hbm, wq_hbm, wkt_hbm, wvt_hbm, wo_hbm, wg_hbm, wu_hbm, wd_hbm, gw_hbm,
               o_hbm,
               x_v, wq_v, wkt_v, wvt_v, wo_v, wg_v, wu_v, wd_v, gw_v, wkv_v,
               k_v, ka_v, vt_v, vn_v, vp_v, g_v, vb_v,
               kb_v, qa_v, qb_v, sh0_v, qs_v, p0_v, sv_v, l0_v, ot_v, acc_v, o_v, sf_v, z_ref, sems):

        def cp(src, dst, k):
            return pltpu.make_async_copy(src, dst, sems.at[k])

        def al(v, m):
            return v if isinstance(v, int) else pl.multiple_of(v, m)

        def x_copy(c):
            rows = pl.ds(al(c * TR, TR), TR)
            return cp(x_hbm.at[rows], x_v.at[rows], c)

        def small_copies():
            return [cp(wkt_hbm, wkt_v, SEM_SMALL), cp(wvt_hbm, wvt_v, SEM_SMALL),
                    cp(gw_hbm, gw_v, SEM_SMALL)]

        def wq_copy(g):
            k = SEM_WQ + g if g < 3 else BODY_SEM[min(g - 3, 1)]
            return cp(wq_hbm.at[:, pl.ds(g * 128, 128)], wq_v.at[g], k)

        def wo_copy(part):
            lo, hi = [(0, 128), (128, D)][part]
            sl = pl.ds(lo, hi - lo)
            return cp(wo_hbm.at[sl], wo_v.at[sl], BODY_SEM[part])

        def body_copies(t):
            out = []
            if t == 0:
                out += [wq_copy(3), wo_copy(0)]
            if t == 1:
                out += [wq_copy(g) for g in range(4, NG)] + [wo_copy(1)]
            if t % RH == 0:
                f = t // RH
                sl = pl.ds(f * FC, FC)
                out += [cp(wg_hbm.at[:, sl], wg_v.at[f], BODY_SEM[t]),
                        cp(wu_hbm.at[:, sl], wu_v.at[f], BODY_SEM[t]),
                        cp(wd_hbm.at[sl], wd_v.at[f], BODY_SEM[t])]
            return out

        def out_copy(tile, lo=0, n=TQ, k=None):
            k = SEM_OUT + tile % 2 if k is None else k
            return cp(o_v.at[tile % 2, pl.ds(lo, n)], o_hbm.at[pl.ds(tile * TQ + lo, n)], k)

        def tie(x, tok, zv):
            bits = pltpu.bitcast(x, I32) | (pltpu.bitcast(tok, I32) & zv)
            return pltpu.bitcast(bits, x.dtype)

        def fold(op, s, r0=None):
            for r in range(s.shape[0] // 8):
                sr = s[r * 8:(r + 1) * 8, :]
                r0 = sr if r0 is None else op(r0, sr)
            return r0

        def qproj_t(tile, g):
            xt = x_v[pl.ds(al(tile * TQ, TQ), TQ), :]
            q = jnp.dot(xt, wq_v[g], preferred_element_type=F32) * qscale
            return q.T.astype(BF16)

        def store_q(qt, row0):
            qf = qt.astype(F32)
            for b in range(LT):
                qa_v[b, row0:row0 + 128, :] = qf[:, b * 128:(b + 1) * 128]

        def spread_q(src8, b, row0):
            for r in range(8):
                qb_v[b, row0 + r] = jnp.broadcast_to(src8[r:r + 1, :], (8, 128))

        def vpu_chain(zv1):
            mrows = []
            prev = None
            for j in range(HPG):
                mx = None
                for kv in range(NV // 8):
                    parts = []
                    for b0 in range(0, LT, 2):
                        accs = [None, None]
                        if prev is not None:
                            tks = [pltpu.bitcast(a, I32) for a in prev]
                            if mx is not None:
                                tks = [tk | pltpu.bitcast(mx[:, (b0 + b) * 128:(b0 + b + 1) * 128], I32)
                                       for b, tk in enumerate(tks)]
                            accs = [pltpu.bitcast(tk & zv1, F32) for tk in tks]
                        for d in range(DH):
                            kk = kb_v[d, kv]
                            for b in range(2):
                                pr = kk * qb_v[b0 + b, j * DH + d]
                                accs[b] = pr if accs[b] is None else accs[b] + pr
                        prev = accs
                        parts += accs
                        for b in range(2):
                            sv_v[j, kv * 8:(kv + 1) * 8, (b0 + b) * 128:(b0 + b + 1) * 128] = accs[b]
                    row = jnp.concatenate(parts, axis=1)
                    mx = row if mx is None else jnp.maximum(mx, row)
                mrows.append(jnp.max(mx, axis=0, keepdims=True))
            return mrows

        def gate_row(tile):
            return jnp.concatenate([g_v[tile * RH + rr][0:1, :] for rr in range(RH)], axis=1)

        def put_ot(u, on):
            for rr in range(RH):
                ot_v[rr, pl.ds(al(u * DH, DH), DH), :] = on[:, rr * TR:(rr + 1) * TR]

        def shift_of(mrow):
            sub = jax.lax.broadcasted_iota(I32, (16, TQ), 0)
            hi = mrow.astype(BF16).astype(F32)
            lo = (mrow - hi).astype(BF16).astype(F32)
            shift = jnp.where(sub == 0, -hi, jnp.where(sub == 1, -lo, 0.0)).astype(BF16)
            return shift, jnp.broadcast_to(hi + lo, (8, TQ))

        def attention(qt, mrows, tile, zv, tail_fn=None, qf_new=None):
            grow = gate_row(tile)
            events = []
            for u in range(HPG):
                for c in range(NC):
                    events.append((u * NC + c, 1, "qk", u, c))
                    events.append((u * NC + c + LAG, 0, "pv", u, c))
            if tail_fn is not None:
                events.append((HPG * NC, 0.5, "tail", 0, 0))
                for g_ in range(NV // 16):
                    events.append((NEXT0 + g_, 0.6, "next", 0, g_))
                for g_ in range((128 - DH) // 8 * LT):
                    events.append((QA0 + g_ * QA_STEP, 0.7, "qa", g_ // LT, g_ % LT))
                for g_ in range(DH // 8 * LT):
                    events.append((QB0 + g_ * QB_STEP, 0.7, "qb", g_ // LT, g_ % LT))
            events.sort()
            s_val, st, nxt = {}, {}, {}
            l_hist, a_hist = [], []
            bad = None
            for _, _, kind, u, c in events:
                if kind == "tail":
                    tail_fn()
                    continue
                if kind in ("qa", "qb"):
                    if kind == "qa":
                        s8 = qa_v[c, 128 + DH + u * 8:128 + DH + (u + 1) * 8, :]
                    else:
                        s8 = qf_new[u * 8:(u + 1) * 8, c * 128:(c + 1) * 128]
                    s8 = tie(s8, l_hist[-1][:, c * 128:(c + 1) * 128], zv[:, :128])
                    spread_q(s8, c, u * 8 + (0 if kind == "qa" else 128 - DH))
                    continue
                if kind == "next":
                    if not nxt:
                        nxt["shift"], nxt["m"] = shift_of(mrows[HPG])
                        nxt["l"] = None
                    m = tie(nxt["m"], l_hist[-2], zv)
                    p = jnp.exp2(sv_v[HPG - 1, c * 16:(c + 1) * 16, :].reshape(2, 8, TQ) - m[None])
                    p = p.reshape(16, TQ)
                    nxt["l"] = fold(jnp.add, p, nxt["l"])
                    p0_v[c * 16:(c + 1) * 16, :] = p
                    if c == NV // 16 - 1:
                        sh0_v[...] = nxt["shift"]
                        l0_v[...] = nxt["l"]
                    continue
                if u not in st:
                    pre = mrows[u] is None
                    shift, mb = (sh0_v[...], l0_v[...]) if pre else shift_of(mrows[u])
                    st[u] = dict(q=qt[u * DH:(u + 1) * DH], shift=shift, m=mb, acc=None,
                                 l=mb if pre else None, pre=pre)
                h = st[u]
                if kind == "qk":
                    k_ = u * NC + c
                    sh = tie(h["shift"], a_hist[k_ - TA], zv) if k_ >= TA else h["shift"]
                    w = jnp.concatenate([h["q"], sh], axis=0)
                    s_val[(u, c)] = jnp.dot(ka_v[pl.ds(*mk[c]), :], w, preferred_element_type=F32)
                    continue
                pv = None
                if vk[c][1]:
                    sc = (p0_v if u == 0 else sv_v.at[u - 1])[pl.ds(*vk[c]), :]
                    if h["pre"]:
                        pv = sc
                    else:
                        pv = jnp.exp2(sc.reshape(vk[c][1] // 8, 8, TQ) - h["m"][None])
                        pv = pv.reshape(vk[c][1], TQ)
                pm = jnp.exp2(s_val.pop((u, c)))
                ls = fold(jnp.add, pm)
                if pv is not None and not h["pre"]:
                    ls = fold(jnp.add, pv, ls)
                groups = [pm[j * 16:(j + 1) * 16] for j in range(mk[c][1] // 16 - 1, -1, -1)]
                if pv is not None:
                    groups = [pv] + groups
                p = jnp.concatenate(groups, axis=0).astype(BF16)
                o = jnp.dot(vp_v[:, pl.ds(c * CK, CK)], p, preferred_element_type=F32)
                h["acc"] = o if h["acc"] is None else h["acc"] + o
                h["l"] = ls if h["l"] is None else h["l"] + ls
                l_hist.append(h["l"])
                a_hist.append(h["acc"][DH - 8:, :])
                if c == NC - 1:
                    lt = jnp.sum(h["l"], axis=0, keepdims=True)
                    put_ot(u, h["acc"] * (grow / lt))
                    ok = jnp.logical_and(lt < 2.0 ** 64, lt > 2.0 ** -64)
                    b_ = jnp.where(ok, 0.0, 1.0)
                    bad = b_ if bad is None else jnp.maximum(bad, b_)
            qs_v[...] = qt
            z_ref[1] = jnp.max(bad).astype(I32) | z_ref[2]

        def exact_attention(tile):
            grow = gate_row(tile)

            def head(u, carry):
                w = qs_v[pl.ds(al(u * DH, DH), DH), :]

                def p1(c, mx):
                    rows = pl.ds(al(c * CK, CK), CK)
                    s = jnp.dot(k_v[rows, :], w, preferred_element_type=F32)
                    sf_v[rows, :] = s
                    return fold(jnp.maximum, s, mx)
                mx = jax.lax.fori_loop(0, NC, p1, jnp.full((8, TQ), -jnp.inf, F32))
                m = jnp.max(mx, axis=0, keepdims=True)

                def p2(c, carry2):
                    acc, l = carry2
                    rows = pl.ds(al(c * CK, CK), CK)
                    p = jnp.exp2(sf_v[rows, :] - m)
                    o = jnp.dot(vt_v[:, rows], p.astype(BF16), preferred_element_type=F32)
                    return acc + o, fold(jnp.add, p, l)
                acc, l = jax.lax.fori_loop(
                    0, NC, p2, (jnp.zeros((DH, TQ), F32), jnp.zeros((8, TQ), F32)))
                put_ot(u, acc * (grow / jnp.sum(l, axis=0, keepdims=True)))
                return carry
            jax.lax.fori_loop(0, HPG, head, 0)

        def fix_up(tile):
            @pl.when(z_ref[1] != 0)
            def _():
                exact_attention(tile)

        def hidden(tile, half, f):
            xt = x_v[pl.ds(al(tile * TQ + half * TR, TR), TR), :]
            gb = jnp.broadcast_to(1.0 - g_v[tile * RH + half][0:1, :], (128, TR)).T
            gg = jnp.dot(xt, wg_v[f], preferred_element_type=F32)
            uu = jnp.dot(xt, wu_v[f], preferred_element_type=F32)
            hh = jnp.maximum(gg, 0.0) * uu
            return jnp.concatenate(
                [hh[:, j * 128:(j + 1) * 128] * gb for j in range(FC // 128)], axis=1).astype(BF16)

        def ffn_part(tile, t):
            f = t >> 1
            wo_g = wo_v[pl.ds(al(t * 128, 128), 128), :]

            def old(row):
                return jnp.where(t > 0, acc_v[pl.ds(row, TR), :], 0.0)

            half = t & 1
            row = al(half * TR, TR)
            o_nat = ot_v[half].T.astype(BF16)
            hh = hidden(tile, half, f)
            y = jnp.dot(o_nat, wo_g, preferred_element_type=F32)
            y = y + jnp.dot(hh, wd_v[f], preferred_element_type=F32)
            y = y + old(row)
            acc_v[pl.ds(row, TR), :] = y
            o_v[tile & 1, pl.ds(row, TR), :] = y.astype(o_v.dtype)

            half1 = (t + 1) & 1
            row1 = al(half1 * TR, TR)
            o_nat1 = ot_v[half1].T.astype(BF16)

            def tail():
                y1 = jnp.dot(o_nat1, wo_g, preferred_element_type=F32)
                acc_v[pl.ds(row1, TR), :] = y1 + old(row1)
            return tail

        z_ref[0] = 0
        z_ref[1] = 0
        for c_ in small_copies():
            c_.start()
        for c in range(RH):
            x_copy(c).start()
        wq_copy(0).start()
        wq_copy(1).start()
        for c in range(RH, XCH):
            x_copy(c).start()
        wq_copy(2).start()
        for t in range(NG):
            for c_ in body_copies(t):
                c_.start()
        for c_ in small_copies():
            c_.wait()
        gw = gw_v[...].astype(F32)
        gw_row = jnp.concatenate([gw[r:r + 1, :] for r in range(D // 128)], axis=1)
        gw16 = jnp.broadcast_to(gw_row, (16, D)).astype(BF16)
        wkv_v[...] = jnp.concatenate([wvt_v[...], gw16, wkt_v[...]], axis=0)

        def kv_chunk(c):
            rows = pl.ds(al(c * TR, TR), TR)
            vt = jax.lax.dot_general(wkv_v[...], x_v[rows, :], NT, preferred_element_type=F32)
            ones = jnp.where(jax.lax.broadcasted_iota(I32, (16, TR), 0) < 2, 1.0, 0.0)
            ka = jnp.concatenate([vt[DH + 16:], ones], axis=0).T
            k_v[rows, :] = ka[:, 0:DH].astype(BF16)
            ka_v[rows, :] = ka.astype(BF16)
            vn_v[rows, :] = vt[:DH].T
            vt_v[:, rows] = vt[:DH].astype(BF16)
            g_v[c] = jax.nn.sigmoid(vt[DH:DH + 8])
            vb_v[c] = jnp.where(fold(jnp.maximum, jnp.abs(vt[:DH])) < 2.0 ** 60, 0.0, 1.0)

        def kb_rows(ds_):
            kf = k_v[0:NV, :].astype(F32)
            for d in ds_:
                kb_v[d] = jnp.broadcast_to(kf[:, d:d + 1], (NV, 128)).reshape(NV // 8, 8, 128)

        def head_start(qh, dst):
            s = jnp.dot(k_v[0:NV, :], qh, preferred_element_type=F32)
            dst[...] = s
            return jnp.max(fold(jnp.maximum, s), axis=0, keepdims=True)

        for c in range(RH):
            x_copy(c).wait()
            kv_chunk(c)
        wq_copy(0).wait()
        qt0 = qproj_t(0, 0)
        mrows = [head_start(qt0[0:DH], p0_v)]
        mrows += [head_start(qt0[j * DH:(j + 1) * DH], sv_v.at[j - 1]) for j in range(1, HPG)]
        kb_rows(range(0, DH // 2))
        x_copy(RH).wait()
        kv_chunk(RH)
        wq_copy(1).wait()
        qt1 = qproj_t(0, 1)
        m_new = head_start(qt1[0:DH], sv_v.at[HPG - 1])
        store_q(qt1, 0)
        kb_rows(range(DH // 2, DH))

        def xbody(cc, carry):
            x_copy(cc).wait()
            kv_chunk(cc)
            return carry
        jax.lax.fori_loop(RH + 1, XCH - 1, xbody, 0)
        x_copy(XCH - 1).wait()
        wq_copy(2).wait()
        kv_chunk(XCH - 1)
        store_q(qproj_t(0, 2), 128)
        for c in range(NC):
            rows_ = [vn_v[pl.ds(mk[c][0] + j * 16, 16), :] for j in range(mk[c][1] // 16 - 1, -1, -1)]
            if vk[c][1]:
                rows_ = [vn_v[pl.ds(*vk[c]), :]] + rows_
            vp_v[:, pl.ds(c * CK, CK)] = jnp.concatenate(rows_, axis=0).T.astype(BF16)
        z_ref[2] = jnp.max(vb_v[...]).astype(I32)
        attention(qt0, mrows, 0, jnp.full((8, TQ), z_ref[0], I32))
        shift, m = shift_of(m_new)
        sh0_v[...] = shift
        p = jnp.exp2(sv_v[HPG - 1].reshape(NV // 8, 8, TQ) - m[None]).reshape(NV, TQ)
        l0_v[...] = fold(jnp.add, p)
        p0_v[...] = p
        for b in range(LT):
            for r in range(0, 128, 8):
                spread_q(qa_v[b, DH + r:DH + r + 8, :], b, r)

        def body(it, carry):
            tile = it >> 3
            t = it & (NG - 1)

            def rare(_, c0):
                for tt in BODY_SEM:
                    @pl.when(it == tt)
                    def _():
                        for c_ in body_copies(tt):
                            c_.wait()
                for q in range(1, NQ):
                    @pl.when(it == q * NG)
                    def _():
                        if q >= 2:
                            out_copy(q - 2).wait()
                        o_v[(q - 1) % 2, 0:TR, :] = acc_v[0:TR, :].astype(o_v.dtype)
                        out_copy(q - 1).start()
                fix_up(tile)
                return c0
            is_rare = jnp.logical_or(jnp.logical_or(it < NG, t == 0), z_ref[1] != 0)
            jax.lax.fori_loop(0, jnp.where(is_rare, 1, 0), rare, 0)

            zv = jnp.full((8, TQ), z_ref[0], I32)
            g3 = jnp.minimum(it + 3, NIT - 1)
            qt_new = qproj_t(g3 >> 3, g3 & (NG - 1))
            mrows = [None] + vpu_chain(zv[:, :128])
            tail_fn = ffn_part(tile, t)
            qt = jnp.concatenate([qa_v[b, 0:128, :] for b in range(LT)], axis=1).astype(BF16)
            attention(qt, mrows, (it + 1) >> 3, zv, tail_fn, qt_new.astype(F32))
            for b in range(LT):
                qa_v[b, 0:128, :] = qa_v[b, 128:256, :]
            store_q(qt_new, 128)
            return carry
        jax.lax.fori_loop(0, NIT - 1, body, 0)
        fix_up(NQ - 1)

        tile, t = NQ - 1, NG - 1
        half = t % RH
        other = 1 - half
        wo_g = wo_v[t * 128:(t + 1) * 128, :]
        hh = hidden(tile, half, t // RH)
        y = jnp.dot(ot_v[other].T.astype(BF16), wo_g, preferred_element_type=F32)
        y = y + acc_v[other * TR:(other + 1) * TR, :]
        o_v[tile % 2, other * TR:(other + 1) * TR, :] = y.astype(o_v.dtype)
        tail = [out_copy(tile, other * TR, TR, SEM_OUT + 2 + ESPLIT)]
        o_nat = ot_v[half].T.astype(BF16)
        tail[0].start()
        ER = TR // ESPLIT
        for e in range(ESPLIT):
            lo = half * TR + e * ER
            y = jnp.dot(o_nat[e * ER:(e + 1) * ER], wo_g, preferred_element_type=F32)
            y = y + jnp.dot(hh[e * ER:(e + 1) * ER], wd_v[t // RH], preferred_element_type=F32)
            y = y + acc_v[lo:lo + ER, :]
            o_v[tile % 2, lo:lo + ER, :] = y.astype(o_v.dtype)
            tail.append(out_copy(tile, lo, ER, SEM_OUT + 2 + e))
            tail[-1].start()
        out_copy(NQ - 2).wait()
        for c_ in tail:
            c_.wait()

    any_spec = pl.BlockSpec(memory_space=pl.ANY)
    out = pl.pallas_call(
        kernel,
        in_specs=[any_spec] * 9,
        out_specs=any_spec,
        out_shape=jax.ShapeDtypeStruct((S, D), A_x.dtype),
        scratch_shapes=[
            pltpu.VMEM((S, D), BF16),
            pltpu.VMEM((NG, D, 128), BF16),
            pltpu.VMEM((DH, D), BF16),
            pltpu.VMEM((DH, D), BF16),
            pltpu.VMEM((D, D), BF16),
            pltpu.VMEM((NF, D, FC), BF16),
            pltpu.VMEM((NF, D, FC), BF16),
            pltpu.VMEM((NF, FC, D), BF16),
            pltpu.VMEM((D // 128, 128), BF16),
            pltpu.VMEM((2 * DH + 16, D), BF16),
            pltpu.VMEM((S, DH), BF16),
            pltpu.VMEM((S, KA), BF16),
            pltpu.VMEM((DH, S), BF16),
            pltpu.VMEM((S, DH), F32),
            pltpu.VMEM((DH, S), BF16),
            pltpu.VMEM((XCH, 8, TR), F32),
            pltpu.VMEM((XCH, 8, TR), F32),
            pltpu.VMEM((DH, NV // 8, 8, 128), F32),
            pltpu.VMEM((LT, 256, 128), F32),
            pltpu.VMEM((LT, 128, 8, 128), F32),
            pltpu.VMEM((16, TQ), BF16),
            pltpu.VMEM((128, TQ), BF16),
            pltpu.VMEM((NV, TQ), F32),
            pltpu.VMEM((HPG, NV, TQ), F32),
            pltpu.VMEM((8, TQ), F32),
            pltpu.VMEM((RH, 128, TR), F32),
            pltpu.VMEM((TQ, D), F32),
            pltpu.VMEM((2, TQ, D), A_x.dtype),
            pltpu.VMEM((S, TQ), F32),
            pltpu.SMEM((3,), I32),
            pltpu.SemaphoreType.DMA((NSEM,)),
        ],
        compiler_params=pltpu.CompilerParams(vmem_limit_bytes=100 * 1024 * 1024),
        name="gated_mix",
    )(A_x.reshape(S, D), A_wq, A_wk.T, A_wv.T, A_wo, B_W_gate, B_W_up, B_W_down,
      gate_w.reshape(D // 128, 128))
    return out.reshape(1, S, D)
```

```python
import math

import jax
import jax.numpy as jnp
import jax.experimental.pallas as pl
import jax.experimental.pallas.tpu as pltpu

F32 = jnp.float32
BF16 = jnp.bfloat16
I32 = jnp.int32
NT = (((1,), (1,)), ((), ()))


TQ = 512
TR = 256
CK = 128
NV = 256
LAG = 2
TA = 3
ESPLIT = 4
NEXT0 = 40
QA0, QA_STEP = 24, 0.7
QB0, QB_STEP = 42, 0.8


@jax.jit
def pallas_gated_mix__grouped_kv_mqa__glu_gated_reglu__prompt_kernel(
    A_x: jax.Array,
    A_wq: jax.Array,
    A_wk: jax.Array,
    A_wv: jax.Array,
    A_wo: jax.Array,
    B_x: jax.Array,
    B_W_gate: jax.Array,
    B_W_up: jax.Array,
    B_W_down: jax.Array,
    gate_w: jax.Array,
):
    del B_x
    _, S, D = A_x.shape
    DH = A_wk.shape[1]
    F = B_W_gate.shape[1]
    HPG = 128 // DH
    NG = D // 128
    NQ = S // TQ
    NIT = NQ * NG
    NC = S // CK
    RH = TQ // TR
    NF = NG // RH
    FC = F // NF
    LT = TQ // 128
    XCH = S // TR
    KA = DH + 16
    qscale = (DH ** -0.5) * math.log2(math.e)
    assert NG == 8 and RH == 2 and LT == 4 and HPG == 4 and FC % 128 == 0
    assert NV % 16 == 0 and NV <= TQ
    ngr = NV // 16
    nvg = [(c + 1) * ngr // NC - c * ngr // NC for c in range(NC)]
    vk = [(sum(nvg[:c]) * 16, nvg[c] * 16) for c in range(NC)]
    mk = [(NV + c * CK - vk[c][0], CK - vk[c][1]) for c in range(NC)]

    SEM_SMALL = XCH
    SEM_WQ = XCH + 1
    SEM_BODY = XCH + 4
    BODY_SEM = {t: SEM_BODY + n
                for n, t in enumerate(t for t in range(NG) if t <= 1 or t % RH == 0)}
    NSEM = SEM_BODY + len(BODY_SEM)
    SEM_OUT = 0

    def kernel(x_hbm, wq_hbm, wkt_hbm, wvt_hbm, wo_hbm, wg_hbm, wu_hbm, wd_hbm, gw_hbm,
               o_hbm,
               x_v, wq_v, wkt_v, wvt_v, wo_v, wg_v, wu_v, wd_v, gw_v, wkv_v,
               k_v, ka_v, vt_v, vn_v, vp_v, g_v, vb_v,
               kb_v, qa_v, qb_v, sh0_v, qs_v, p0_v, sv_v, l0_v, ot_v, acc_v, o_v, sf_v, z_ref, sems):

        def cp(src, dst, k):
            return pltpu.make_async_copy(src, dst, sems.at[k])

        def al(v, m):
            return v if isinstance(v, int) else pl.multiple_of(v, m)

        def x_copy(c):
            rows = pl.ds(al(c * TR, TR), TR)
            return cp(x_hbm.at[rows], x_v.at[rows], c)

        def small_copies():
            return [cp(wkt_hbm, wkt_v, SEM_SMALL), cp(wvt_hbm, wvt_v, SEM_SMALL),
                    cp(gw_hbm, gw_v, SEM_SMALL)]

        def wq_copy(g):
            k = SEM_WQ + g if g < 3 else BODY_SEM[min(g - 3, 1)]
            return cp(wq_hbm.at[:, pl.ds(g * 128, 128)], wq_v.at[g], k)

        def wo_copy(part):
            lo, hi = [(0, 128), (128, D)][part]
            sl = pl.ds(lo, hi - lo)
            return cp(wo_hbm.at[sl], wo_v.at[sl], BODY_SEM[part])

        def body_copies(t):
            out = []
            if t == 0:
                out += [wq_copy(3), wo_copy(0)]
            if t == 1:
                out += [wq_copy(g) for g in range(4, NG)] + [wo_copy(1)]
            if t % RH == 0:
                f = t // RH
                sl = pl.ds(f * FC, FC)
                out += [cp(wg_hbm.at[:, sl], wg_v.at[f], BODY_SEM[t]),
                        cp(wu_hbm.at[:, sl], wu_v.at[f], BODY_SEM[t]),
                        cp(wd_hbm.at[sl], wd_v.at[f], BODY_SEM[t])]
            return out

        def out_copy(tile, lo=0, n=TQ, k=None):
            k = SEM_OUT + tile % 2 if k is None else k
            return cp(o_v.at[tile % 2, pl.ds(lo, n)], o_hbm.at[pl.ds(tile * TQ + lo, n)], k)

        def tie(x, tok, zv):
            bits = pltpu.bitcast(x, I32) | (pltpu.bitcast(tok, I32) & zv)
            return pltpu.bitcast(bits, x.dtype)

        def fold(op, s, r0=None):
            for r in range(s.shape[0] // 8):
                sr = s[r * 8:(r + 1) * 8, :]
                r0 = sr if r0 is None else op(r0, sr)
            return r0

        def qproj_t(tile, g):
            xt = x_v[pl.ds(al(tile * TQ, TQ), TQ), :]
            q = jnp.dot(xt, wq_v[g], preferred_element_type=F32) * qscale
            return q.T.astype(BF16)

        def store_q(qt, row0):
            qf = qt.astype(F32)
            for b in range(LT):
                qa_v[b, row0:row0 + 128, :] = qf[:, b * 128:(b + 1) * 128]

        def spread_q(src8, b, row0):
            for r in range(8):
                qb_v[b, row0 + r] = jnp.broadcast_to(src8[r:r + 1, :], (8, 128))

        def vpu_chain(zv1):
            def row_step(j, kv, prev, mx):
                parts = []
                for b0 in range(0, LT, 2):
                    def prod(d, b):
                        return kb_v[d, kv] * qb_v[b0 + b, j * DH + d]

                    def mac(d, accs):
                        kk = kb_v[d, kv]
                        return tuple(accs[b] + kk * qb_v[b0 + b, j * DH + d] for b in range(2))
                    if prev is None:
                        prev = jax.lax.fori_loop(1, DH, mac, (prod(0, 0), prod(0, 1)), unroll=True)
                    else:
                        tks = [pltpu.bitcast(a, I32) for a in prev]
                        if mx is not None:
                            tks = [tk | pltpu.bitcast(mx[:, (b0 + b) * 128:(b0 + b + 1) * 128], I32)
                                   for b, tk in enumerate(tks)]
                        init = tuple(pltpu.bitcast(tk & zv1, F32) for tk in tks)
                        prev = jax.lax.fori_loop(0, DH, mac, init, unroll=True)
                    parts += prev
                    for b in range(2):
                        sv_v[j, pl.ds(al(kv * 8, 8), 8), (b0 + b) * 128:(b0 + b + 1) * 128] = prev[b]
                row = jnp.concatenate(parts, axis=1)
                return prev, row if mx is None else jnp.maximum(mx, row)

            mrows = []
            prev = None
            for j in range(HPG):
                prev, mx = jax.lax.fori_loop(
                    1, NV // 8, lambda kv, c, j=j: row_step(j, kv, *c), row_step(j, 0, prev, None),
                    unroll=True)
                mrows.append(jnp.max(mx, axis=0, keepdims=True))
            return mrows

        def gate_row(tile):
            return jnp.concatenate([g_v[tile * RH + rr][0:1, :] for rr in range(RH)], axis=1)

        def put_ot(u, on):
            for rr in range(RH):
                ot_v[rr, pl.ds(al(u * DH, DH), DH), :] = on[:, rr * TR:(rr + 1) * TR]

        def shift_of(mrow):
            sub = jax.lax.broadcasted_iota(I32, (16, TQ), 0)
            hi = mrow.astype(BF16).astype(F32)
            lo = (mrow - hi).astype(BF16).astype(F32)
            shift = jnp.where(sub == 0, -hi, jnp.where(sub == 1, -lo, 0.0)).astype(BF16)
            return shift, jnp.broadcast_to(hi + lo, (8, TQ))

        def attention(qt, mrows, tile, zv, tail_fn=None, qf_new=None):
            grow = gate_row(tile)
            events = []
            for u in range(HPG):
                for c in range(NC):
                    events.append((u * NC + c, 1, "qk", u, c))
                    events.append((u * NC + c + LAG, 0, "pv", u, c))
            if tail_fn is not None:
                events.append((HPG * NC, 0.5, "tail", 0, 0))
                for g_ in range(NV // 16):
                    events.append((NEXT0 + g_, 0.6, "next", 0, g_))
                for g_ in range((128 - DH) // 8 * LT):
                    events.append((QA0 + g_ * QA_STEP, 0.7, "qa", g_ // LT, g_ % LT))
                for g_ in range(DH // 8 * LT):
                    events.append((QB0 + g_ * QB_STEP, 0.7, "qb", g_ // LT, g_ % LT))
            events.sort()
            s_val, st, nxt = {}, {}, {}
            l_hist, a_hist = [], []
            bad = None
            for _, _, kind, u, c in events:
                if kind == "tail":
                    tail_fn()
                    continue
                if kind in ("qa", "qb"):
                    if kind == "qa":
                        s8 = qa_v[c, 128 + DH + u * 8:128 + DH + (u + 1) * 8, :]
                    else:
                        s8 = qf_new[u * 8:(u + 1) * 8, c * 128:(c + 1) * 128]
                    s8 = tie(s8, l_hist[-1][:, c * 128:(c + 1) * 128], zv[:, :128])
                    spread_q(s8, c, u * 8 + (0 if kind == "qa" else 128 - DH))
                    continue
                if kind == "next":
                    if not nxt:
                        nxt["shift"], nxt["m"] = shift_of(mrows[HPG])
                        nxt["l"] = None
                    m = tie(nxt["m"], l_hist[-2], zv)
                    p = jnp.exp2(sv_v[HPG - 1, c * 16:(c + 1) * 16, :].reshape(2, 8, TQ) - m[None])
                    p = p.reshape(16, TQ)
                    nxt["l"] = fold(jnp.add, p, nxt["l"])
                    p0_v[c * 16:(c + 1) * 16, :] = p
                    if c == NV // 16 - 1:
                        sh0_v[...] = nxt["shift"]
                        l0_v[...] = nxt["l"]
                    continue
                if u not in st:
                    pre = mrows[u] is None
                    shift, mb = (sh0_v[...], l0_v[...]) if pre else shift_of(mrows[u])
                    st[u] = dict(q=qt[u * DH:(u + 1) * DH], shift=shift, m=mb, acc=None,
                                 l=mb if pre else None, pre=pre)
                h = st[u]
                if kind == "qk":
                    k_ = u * NC + c
                    sh = tie(h["shift"], a_hist[k_ - TA], zv) if k_ >= TA else h["shift"]
                    w = jnp.concatenate([h["q"], sh], axis=0)
                    s_val[(u, c)] = jnp.dot(ka_v[pl.ds(*mk[c]), :], w, preferred_element_type=F32)
                    continue
                pv = None
                if vk[c][1]:
                    sc = (p0_v if u == 0 else sv_v.at[u - 1])[pl.ds(*vk[c]), :]
                    if h["pre"]:
                        pv = sc
                    else:
                        pv = jnp.exp2(sc.reshape(vk[c][1] // 8, 8, TQ) - h["m"][None])
                        pv = pv.reshape(vk[c][1], TQ)
                pm = jnp.exp2(s_val.pop((u, c)))
                ls = fold(jnp.add, pm)
                if pv is not None and not h["pre"]:
                    ls = fold(jnp.add, pv, ls)
                groups = [pm[j * 16:(j + 1) * 16] for j in range(mk[c][1] // 16 - 1, -1, -1)]
                if pv is not None:
                    groups = [pv] + groups
                p = jnp.concatenate(groups, axis=0).astype(BF16)
                o = jnp.dot(vp_v[:, pl.ds(c * CK, CK)], p, preferred_element_type=F32)
                h["acc"] = o if h["acc"] is None else h["acc"] + o
                h["l"] = ls if h["l"] is None else h["l"] + ls
                l_hist.append(h["l"])
                a_hist.append(h["acc"][DH - 8:, :])
                if c == NC - 1:
                    lt = jnp.sum(h["l"], axis=0, keepdims=True)
                    put_ot(u, h["acc"] * (grow / lt))
                    ok = jnp.logical_and(lt < 2.0 ** 64, lt > 2.0 ** -64)
                    b_ = jnp.where(ok, 0.0, 1.0)
                    bad = b_ if bad is None else jnp.maximum(bad, b_)
            qs_v[...] = qt
            z_ref[1] = jnp.max(bad).astype(I32) | z_ref[2]

        def exact_attention(tile):
            grow = gate_row(tile)

            def head(u, carry):
                w = qs_v[pl.ds(al(u * DH, DH), DH), :]

                def p1(c, mx):
                    rows = pl.ds(al(c * CK, CK), CK)
                    s = jnp.dot(k_v[rows, :], w, preferred_element_type=F32)
                    sf_v[rows, :] = s
                    return fold(jnp.maximum, s, mx)
                mx = jax.lax.fori_loop(0, NC, p1, jnp.full((8, TQ), -jnp.inf, F32))
                m = jnp.max(mx, axis=0, keepdims=True)

                def p2(c, carry2):
                    acc, l = carry2
                    rows = pl.ds(al(c * CK, CK), CK)
                    p = jnp.exp2(sf_v[rows, :] - m)
                    o = jnp.dot(vt_v[:, rows], p.astype(BF16), preferred_element_type=F32)
                    return acc + o, fold(jnp.add, p, l)
                acc, l = jax.lax.fori_loop(
                    0, NC, p2, (jnp.zeros((DH, TQ), F32), jnp.zeros((8, TQ), F32)))
                put_ot(u, acc * (grow / jnp.sum(l, axis=0, keepdims=True)))
                return carry
            jax.lax.fori_loop(0, HPG, head, 0)

        def fix_up(tile):
            @pl.when(z_ref[1] != 0)
            def _():
                exact_attention(tile)

        def hidden(tile, half, f):
            xt = x_v[pl.ds(al(tile * TQ + half * TR, TR), TR), :]
            gb = jnp.broadcast_to(1.0 - g_v[tile * RH + half][0:1, :], (128, TR)).T
            gg = jnp.dot(xt, wg_v[f], preferred_element_type=F32)
            uu = jnp.dot(xt, wu_v[f], preferred_element_type=F32)
            hh = jnp.maximum(gg, 0.0) * uu
            return jnp.concatenate(
                [hh[:, j * 128:(j + 1) * 128] * gb for j in range(FC // 128)], axis=1).astype(BF16)

        def ffn_part(tile, t):
            f = t >> 1
            wo_g = wo_v[pl.ds(al(t * 128, 128), 128), :]

            def old(row):
                return jnp.where(t > 0, acc_v[pl.ds(row, TR), :], 0.0)

            half = t & 1
            row = al(half * TR, TR)
            o_nat = ot_v[half].T.astype(BF16)
            hh = hidden(tile, half, f)
            y = jnp.dot(o_nat, wo_g, preferred_element_type=F32)
            y = y + jnp.dot(hh, wd_v[f], preferred_element_type=F32)
            y = y + old(row)
            acc_v[pl.ds(row, TR), :] = y
            o_v[tile & 1, pl.ds(row, TR), :] = y.astype(o_v.dtype)

            half1 = (t + 1) & 1
            row1 = al(half1 * TR, TR)
            o_nat1 = ot_v[half1].T.astype(BF16)

            def tail():
                y1 = jnp.dot(o_nat1, wo_g, preferred_element_type=F32)
                acc_v[pl.ds(row1, TR), :] = y1 + old(row1)
            return tail

        z_ref[0] = 0
        z_ref[1] = 0
        for c_ in small_copies():
            c_.start()
        for c in range(RH):
            x_copy(c).start()
        wq_copy(0).start()
        wq_copy(1).start()
        for c in range(RH, XCH):
            x_copy(c).start()
        wq_copy(2).start()
        for t in range(NG):
            for c_ in body_copies(t):
                c_.start()
        for c_ in small_copies():
            c_.wait()
        gw = gw_v[...].astype(F32)
        gw_row = jnp.concatenate([gw[r:r + 1, :] for r in range(D // 128)], axis=1)
        gw16 = jnp.broadcast_to(gw_row, (16, D)).astype(BF16)
        wkv_v[...] = jnp.concatenate([wvt_v[...], gw16, wkt_v[...]], axis=0)

        def kv_chunk(c):
            rows = pl.ds(al(c * TR, TR), TR)
            vt = jax.lax.dot_general(wkv_v[...], x_v[rows, :], NT, preferred_element_type=F32)
            ones = jnp.where(jax.lax.broadcasted_iota(I32, (16, TR), 0) < 2, 1.0, 0.0)
            ka = jnp.concatenate([vt[DH + 16:], ones], axis=0).T
            k_v[rows, :] = ka[:, 0:DH].astype(BF16)
            ka_v[rows, :] = ka.astype(BF16)
            vn_v[rows, :] = vt[:DH].T
            vt_v[:, rows] = vt[:DH].astype(BF16)
            g_v[c] = jax.nn.sigmoid(vt[DH:DH + 8])
            vb_v[c] = jnp.where(fold(jnp.maximum, jnp.abs(vt[:DH])) < 2.0 ** 60, 0.0, 1.0)

        def kb_rows(ds_):
            kf = k_v[0:NV, :].astype(F32)
            for d in ds_:
                kb_v[d] = jnp.broadcast_to(kf[:, d:d + 1], (NV, 128)).reshape(NV // 8, 8, 128)

        def head_start(qh, dst):
            s = jnp.dot(k_v[0:NV, :], qh, preferred_element_type=F32)
            dst[...] = s
            return jnp.max(fold(jnp.maximum, s), axis=0, keepdims=True)

        for c in range(RH):
            x_copy(c).wait()
            kv_chunk(c)
        wq_copy(0).wait()
        qt0 = qproj_t(0, 0)
        mrows = [head_start(qt0[0:DH], p0_v)]
        mrows += [head_start(qt0[j * DH:(j + 1) * DH], sv_v.at[j - 1]) for j in range(1, HPG)]
        kb_rows(range(0, DH // 2))
        x_copy(RH).wait()
        kv_chunk(RH)
        wq_copy(1).wait()
        qt1 = qproj_t(0, 1)
        m_new = head_start(qt1[0:DH], sv_v.at[HPG - 1])
        store_q(qt1, 0)
        kb_rows(range(DH // 2, DH))

        def xbody(cc, carry):
            x_copy(cc).wait()
            kv_chunk(cc)
            return carry
        jax.lax.fori_loop(RH + 1, XCH - 1, xbody, 0)
        x_copy(XCH - 1).wait()
        wq_copy(2).wait()
        kv_chunk(XCH - 1)
        store_q(qproj_t(0, 2), 128)
        for c in range(NC):
            rows_ = [vn_v[pl.ds(mk[c][0] + j * 16, 16), :] for j in range(mk[c][1] // 16 - 1, -1, -1)]
            if vk[c][1]:
                rows_ = [vn_v[pl.ds(*vk[c]), :]] + rows_
            vp_v[:, pl.ds(c * CK, CK)] = jnp.concatenate(rows_, axis=0).T.astype(BF16)
        z_ref[2] = jnp.max(vb_v[...]).astype(I32)
        attention(qt0, mrows, 0, jnp.full((8, TQ), z_ref[0], I32))
        shift, m = shift_of(m_new)
        sh0_v[...] = shift
        p = jnp.exp2(sv_v[HPG - 1].reshape(NV // 8, 8, TQ) - m[None]).reshape(NV, TQ)
        l0_v[...] = fold(jnp.add, p)
        p0_v[...] = p
        for b in range(LT):
            for r in range(0, 128, 8):
                spread_q(qa_v[b, DH + r:DH + r + 8, :], b, r)

        def body(it, carry):
            tile = it >> 3
            t = it & (NG - 1)

            def rare(_, c0):
                for tt in BODY_SEM:
                    @pl.when(it == tt)
                    def _():
                        for c_ in body_copies(tt):
                            c_.wait()
                for q in range(1, NQ):
                    @pl.when(it == q * NG)
                    def _():
                        if q >= 2:
                            out_copy(q - 2).wait()
                        o_v[(q - 1) % 2, 0:TR, :] = acc_v[0:TR, :].astype(o_v.dtype)
                        out_copy(q - 1).start()
                fix_up(tile)
                return c0
            is_rare = jnp.logical_or(jnp.logical_or(it < NG, t == 0), z_ref[1] != 0)
            jax.lax.fori_loop(0, jnp.where(is_rare, 1, 0), rare, 0)

            zv = jnp.full((8, TQ), z_ref[0], I32)
            g3 = jnp.minimum(it + 3, NIT - 1)
            qt_new = qproj_t(g3 >> 3, g3 & (NG - 1))
            mrows = [None] + vpu_chain(zv[:, :128])
            tail_fn = ffn_part(tile, t)
            qt = jnp.concatenate([qa_v[b, 0:128, :] for b in range(LT)], axis=1).astype(BF16)
            attention(qt, mrows, (it + 1) >> 3, zv, tail_fn, qt_new.astype(F32))
            for b in range(LT):
                qa_v[b, 0:128, :] = qa_v[b, 128:256, :]
            store_q(qt_new, 128)
            return carry
        jax.lax.fori_loop(0, NIT - 1, body, 0)
        fix_up(NQ - 1)

        tile, t = NQ - 1, NG - 1
        half = t % RH
        other = 1 - half
        wo_g = wo_v[t * 128:(t + 1) * 128, :]
        hh = hidden(tile, half, t // RH)
        y = jnp.dot(ot_v[other].T.astype(BF16), wo_g, preferred_element_type=F32)
        y = y + acc_v[other * TR:(other + 1) * TR, :]
        o_v[tile % 2, other * TR:(other + 1) * TR, :] = y.astype(o_v.dtype)
        tail = [out_copy(tile, other * TR, TR, SEM_OUT + 2 + ESPLIT)]
        o_nat = ot_v[half].T.astype(BF16)
        tail[0].start()
        ER = TR // ESPLIT
        for e in range(ESPLIT):
            lo = half * TR + e * ER
            y = jnp.dot(o_nat[e * ER:(e + 1) * ER], wo_g, preferred_element_type=F32)
            y = y + jnp.dot(hh[e * ER:(e + 1) * ER], wd_v[t // RH], preferred_element_type=F32)
            y = y + acc_v[lo:lo + ER, :]
            o_v[tile % 2, lo:lo + ER, :] = y.astype(o_v.dtype)
            tail.append(out_copy(tile, lo, ER, SEM_OUT + 2 + e))
            tail[-1].start()
        out_copy(NQ - 2).wait()
        for c_ in tail:
            c_.wait()

    any_spec = pl.BlockSpec(memory_space=pl.ANY)
    out = pl.pallas_call(
        kernel,
        in_specs=[any_spec] * 9,
        out_specs=any_spec,
        out_shape=jax.ShapeDtypeStruct((S, D), A_x.dtype),
        scratch_shapes=[
            pltpu.VMEM((S, D), BF16),
            pltpu.VMEM((NG, D, 128), BF16),
            pltpu.VMEM((DH, D), BF16),
            pltpu.VMEM((DH, D), BF16),
            pltpu.VMEM((D, D), BF16),
            pltpu.VMEM((NF, D, FC), BF16),
            pltpu.VMEM((NF, D, FC), BF16),
            pltpu.VMEM((NF, FC, D), BF16),
            pltpu.VMEM((D // 128, 128), BF16),
            pltpu.VMEM((2 * DH + 16, D), BF16),
            pltpu.VMEM((S, DH), BF16),
            pltpu.VMEM((S, KA), BF16),
            pltpu.VMEM((DH, S), BF16),
            pltpu.VMEM((S, DH), F32),
            pltpu.VMEM((DH, S), BF16),
            pltpu.VMEM((XCH, 8, TR), F32),
            pltpu.VMEM((XCH, 8, TR), F32),
            pltpu.VMEM((DH, NV // 8, 8, 128), F32),
            pltpu.VMEM((LT, 256, 128), F32),
            pltpu.VMEM((LT, 128, 8, 128), F32),
            pltpu.VMEM((16, TQ), BF16),
            pltpu.VMEM((128, TQ), BF16),
            pltpu.VMEM((NV, TQ), F32),
            pltpu.VMEM((HPG, NV, TQ), F32),
            pltpu.VMEM((8, TQ), F32),
            pltpu.VMEM((RH, 128, TR), F32),
            pltpu.VMEM((TQ, D), F32),
            pltpu.VMEM((2, TQ, D), A_x.dtype),
            pltpu.VMEM((S, TQ), F32),
            pltpu.SMEM((3,), I32),
            pltpu.SemaphoreType.DMA((NSEM,)),
        ],
        compiler_params=pltpu.CompilerParams(vmem_limit_bytes=100 * 1024 * 1024),
        name="gated_mix",
    )(A_x.reshape(S, D), A_wq, A_wk.T, A_wv.T, A_wo, B_W_gate, B_W_up, B_W_down,
      gate_w.reshape(D // 128, 128))
    return out.reshape(1, S, D)
```

```python
import math

import jax
import jax.numpy as jnp
import jax.experimental.pallas as pl
import jax.experimental.pallas.tpu as pltpu

F32 = jnp.float32
BF16 = jnp.bfloat16
I32 = jnp.int32
NT = (((1,), (1,)), ((), ()))

TQ = 512
TR = 256
CK = 128
NV = 256
LAG = 2
TA = 3
PA = 6
ESPLIT = 4
NEXT0 = 40
QA0, QA_STEP = 24, 0.7
QB0, QB_STEP = 42, 0.8


@jax.jit
def pallas_gated_mix__grouped_kv_mqa__glu_gated_reglu__prompt_kernel(
    A_x: jax.Array,
    A_wq: jax.Array,
    A_wk: jax.Array,
    A_wv: jax.Array,
    A_wo: jax.Array,
    B_x: jax.Array,
    B_W_gate: jax.Array,
    B_W_up: jax.Array,
    B_W_down: jax.Array,
    gate_w: jax.Array,
):
    del B_x
    _, S, D = A_x.shape
    DH = A_wk.shape[1]
    F = B_W_gate.shape[1]
    HPG = 128 // DH
    NG = D // 128
    NQ = S // TQ
    NIT = NQ * NG
    NC = S // CK
    RH = TQ // TR
    NF = NG // RH
    FC = F // NF
    LT = TQ // 128
    XCH = S // TR
    KA = DH + 16
    qscale = (DH ** -0.5) * math.log2(math.e)
    assert NQ == 4 and NG == 8 and RH == 2 and LT == 4 and HPG == 4 and FC % 128 == 0
    assert NV % 16 == 0 and NV <= TQ and NQ + ESPLIT <= XCH
    ngr = NV // 16
    nvg = [(c + 1) * ngr // NC - c * ngr // NC for c in range(NC)]
    vk = [(sum(nvg[:c]) * 16, nvg[c] * 16) for c in range(NC)]
    mk = [(NV + c * CK - vk[c][0], CK - vk[c][1]) for c in range(NC)]

    SEM_SMALL = XCH
    SEM_WQ = XCH + 1
    SEM_BODY = XCH + 2
    BODY_SEM = {it: SEM_BODY + n
                for n, it in enumerate([0, 1] + [f * RH * NQ for f in range(1, NF)])}
    NSEM = SEM_BODY + len(BODY_SEM)
    SEM_OUT = 0

    def kernel(x_hbm, wq_hbm, wkt_hbm, wvt_hbm, wo_hbm, wg_hbm, wu_hbm, wd_hbm, gw_hbm,
               o_hbm,
               x_v, wq_v, wkt_v, wvt_v, wo_v, wg_v, wu_v, wd_v, gw_v, wkv_v,
               k_v, ka_v, vt_v, vn_v, vp_v, g_v, vb_v,
               kb_v, qa_v, qb_v, sh0_v, qs_v, p0_v, sv_v, l0_v, ot_v, acc_v, o_v, sf_v, z_ref, sems):

        def cp(src, dst, k):
            return pltpu.make_async_copy(src, dst, sems.at[k])

        def al(v, m):
            return v if isinstance(v, int) else pl.multiple_of(v, m)

        def x_copy(c):
            rows = pl.ds(al(c * TR, TR), TR)
            return cp(x_hbm.at[rows], x_v.at[rows], c)

        def small_copies():
            return [cp(wkt_hbm, wkt_v, SEM_SMALL), cp(wvt_hbm, wvt_v, SEM_SMALL),
                    cp(gw_hbm, gw_v, SEM_SMALL)]

        def wq_copy(g):
            k = SEM_WQ if g == 0 else BODY_SEM[1]
            return cp(wq_hbm.at[:, pl.ds(g * 128, 128)], wq_v.at[g], k)

        def wo_copy(part):
            lo, hi = [(0, 128), (128, D)][part]
            sl = pl.ds(lo, hi - lo)
            return cp(wo_hbm.at[sl], wo_v.at[sl], BODY_SEM[part])

        def body_copies(t):
            out = []
            if t == 0:
                out += [wo_copy(0)]
            if t == 1:
                out += [wq_copy(g) for g in range(1, NG)] + [wo_copy(1)]
            if t % (RH * NQ) == 0:
                f = t // (RH * NQ)
                sl = pl.ds(f * FC, FC)
                out += [cp(wg_hbm.at[:, sl], wg_v.at[f], BODY_SEM[t]),
                        cp(wu_hbm.at[:, sl], wu_v.at[f], BODY_SEM[t]),
                        cp(wd_hbm.at[sl], wd_v.at[f], BODY_SEM[t])]
            return out

        def out_copy(tile, lo=0, n=TQ, k=None):
            k = SEM_OUT + tile if k is None else k
            rows = pl.ds(tile * TQ + lo, n)
            return cp(o_v.at[rows], o_hbm.at[rows], k)

        def tie(x, tok, zv):
            bits = pltpu.bitcast(x, I32) | (pltpu.bitcast(tok, I32) & zv)
            return pltpu.bitcast(bits, x.dtype)

        def fold(op, s, r0=None):
            for r in range(s.shape[0] // 8):
                sr = s[r * 8:(r + 1) * 8, :]
                r0 = sr if r0 is None else op(r0, sr)
            return r0

        def qproj_t(tile, g):
            xt = x_v[pl.ds(al(tile * TQ, TQ), TQ), :]
            q = jnp.dot(xt, wq_v[g], preferred_element_type=F32) * qscale
            return q.T.astype(BF16)

        def store_q(qt, row0):
            qf = qt.astype(F32)
            for b in range(LT):
                qa_v[b, row0:row0 + 128, :] = qf[:, b * 128:(b + 1) * 128]

        def spread_q(src8, b, row0):
            for r in range(8):
                qb_v[b, row0 + r] = jnp.broadcast_to(src8[r:r + 1, :], (8, 128))

        def vpu_chain(zv1):
            def row_step(j, kv, prev, mx):
                parts = []
                for b0 in range(0, LT, 2):
                    def prod(d, b):
                        return kb_v[d, kv] * qb_v[b0 + b, j * DH + d]

                    def mac(d, accs):
                        kk = kb_v[d, kv]
                        return tuple(accs[b] + kk * qb_v[b0 + b, j * DH + d] for b in range(2))
                    if prev is None:
                        prev = jax.lax.fori_loop(1, DH, mac, (prod(0, 0), prod(0, 1)), unroll=True)
                    else:
                        tks = [pltpu.bitcast(a, I32) for a in prev]
                        if mx is not None:
                            tks = [tk | pltpu.bitcast(mx[:, (b0 + b) * 128:(b0 + b + 1) * 128], I32)
                                   for b, tk in enumerate(tks)]
                        init = tuple(pltpu.bitcast(tk & zv1, F32) for tk in tks)
                        prev = jax.lax.fori_loop(0, DH, mac, init, unroll=True)
                    parts += prev
                    for b in range(2):
                        sv_v[j, pl.ds(al(kv * 8, 8), 8), (b0 + b) * 128:(b0 + b + 1) * 128] = prev[b]
                row = jnp.concatenate(parts, axis=1)
                return prev, row if mx is None else jnp.maximum(mx, row)

            mrows = []
            prev = None
            for j in range(HPG):
                prev, mx = jax.lax.fori_loop(
                    1, NV // 8, lambda kv, c, j=j: row_step(j, kv, *c), row_step(j, 0, prev, None),
                    unroll=True)
                mrows.append(jnp.max(mx, axis=0, keepdims=True))
            return mrows

        def gate_row(tile):
            return jnp.concatenate([g_v[tile * RH + rr][0:1, :] for rr in range(RH)], axis=1)

        def put_ot(u, on):
            for rr in range(RH):
                ot_v[rr, pl.ds(al(u * DH, DH), DH), :] = on[:, rr * TR:(rr + 1) * TR]

        def shift_of(mrow):
            sub = jax.lax.broadcasted_iota(I32, (16, TQ), 0)
            hi = mrow.astype(BF16).astype(F32)
            lo = (mrow - hi).astype(BF16).astype(F32)
            shift = jnp.where(sub == 0, -hi, jnp.where(sub == 1, -lo, 0.0)).astype(BF16)
            return shift, jnp.broadcast_to(hi + lo, (8, TQ))

        def attention(qt, mrows, tile, zv, tail_fn=None, qf_new=None, tiles=None, st=None):
            grow = gate_row(tile)
            events = []
            tiles = list(range(NC)) if tiles is None else tiles
            for u in range(HPG):
                for n_, c in enumerate(tiles):
                    events.append((u * len(tiles) + n_, 1, "qk", u, c))
                    events.append((u * len(tiles) + n_ + LAG, 0, "pv", u, c))
            if tail_fn is not None:
                events.append((HPG * NC, 0.5, "tail", 0, 0))
                for g_ in range(NV // 16):
                    events.append((NEXT0 + g_, 0.6, "next", 0, g_))
                for g_ in range((128 - DH) // 8 * LT):
                    events.append((QA0 + g_ * QA_STEP, 0.7, "qa", g_ // LT, g_ % LT))
                for g_ in range(DH // 8 * LT):
                    events.append((QB0 + g_ * QB_STEP, 0.7, "qb", g_ // LT, g_ % LT))
            events.sort()
            s_val, nxt = {}, {}
            st = {} if st is None else st
            nqk = 0
            l_hist, a_hist = [], []
            bad = None
            for _, _, kind, u, c in events:
                if kind == "tail":
                    tail_fn()
                    continue
                if kind in ("qa", "qb"):
                    if kind == "qa":
                        s8 = qa_v[c, 128 + DH + u * 8:128 + DH + (u + 1) * 8, :]
                    else:
                        s8 = qf_new[u * 8:(u + 1) * 8, c * 128:(c + 1) * 128]
                    s8 = tie(s8, l_hist[-1][:, c * 128:(c + 1) * 128], zv[:, :128])
                    spread_q(s8, c, u * 8 + (0 if kind == "qa" else 128 - DH))
                    continue
                if kind == "next":
                    if not nxt:
                        nxt["shift"], nxt["m"] = shift_of(mrows[HPG])
                        nxt["l"] = None
                    m = tie(nxt["m"], l_hist[-2], zv)
                    p = jnp.exp2(sv_v[HPG - 1, c * 16:(c + 1) * 16, :].reshape(2, 8, TQ) - m[None])
                    p = p.reshape(16, TQ)
                    nxt["l"] = fold(jnp.add, p, nxt["l"])
                    p0_v[c * 16:(c + 1) * 16, :] = p
                    if c == NV // 16 - 1:
                        sh0_v[...] = nxt["shift"]
                        l0_v[...] = nxt["l"]
                    continue
                if u not in st:
                    pre = mrows[u] is None
                    shift, mb = (sh0_v[...], l0_v[...]) if pre else shift_of(mrows[u])
                    st[u] = dict(q=qt[u * DH:(u + 1) * DH], shift=shift, m=mb, acc=None,
                                 l=mb if pre else None, pre=pre)
                h = st[u]
                if kind == "qk":
                    sh = tie(h["shift"], a_hist[nqk - TA], zv) if nqk >= TA else h["shift"]
                    nqk += 1
                    w = jnp.concatenate([h["q"], sh], axis=0)
                    s_val[(u, c)] = jnp.dot(ka_v[pl.ds(*mk[c]), :], w, preferred_element_type=F32)
                    continue
                pv = None
                if vk[c][1]:
                    sc = (p0_v if u == 0 else sv_v.at[u - 1])[pl.ds(*vk[c]), :]
                    if h["pre"]:
                        pv = sc
                    else:
                        pv = jnp.exp2(sc.reshape(vk[c][1] // 8, 8, TQ) - h["m"][None])
                        pv = pv.reshape(vk[c][1], TQ)
                pm = jnp.exp2(s_val.pop((u, c)))
                ls = fold(jnp.add, pm)
                if pv is not None and not h["pre"]:
                    ls = fold(jnp.add, pv, ls)
                groups = [pm[j * 16:(j + 1) * 16] for j in range(mk[c][1] // 16 - 1, -1, -1)]
                if pv is not None:
                    groups = [pv] + groups
                p = jnp.concatenate(groups, axis=0).astype(BF16)
                o = jnp.dot(vp_v[:, pl.ds(c * CK, CK)], p, preferred_element_type=F32)
                h["acc"] = o if h["acc"] is None else h["acc"] + o
                h["l"] = ls if h["l"] is None else h["l"] + ls
                l_hist.append(h["l"])
                a_hist.append(h["acc"][DH - 8:, :])
                if c == NC - 1:
                    lt = jnp.sum(h["l"], axis=0, keepdims=True)
                    put_ot(u, h["acc"] * (grow / lt))
                    ok = jnp.logical_and(lt < 2.0 ** 64, lt > 2.0 ** -64)
                    b_ = jnp.where(ok, 0.0, 1.0)
                    bad = b_ if bad is None else jnp.maximum(bad, b_)
            if bad is not None:
                qs_v[...] = qt
                z_ref[1] = jnp.max(bad).astype(I32) | z_ref[2]
            return st

        def exact_attention(tile):
            grow = gate_row(tile)

            def head(u, carry):
                w = qs_v[pl.ds(al(u * DH, DH), DH), :]

                def p1(c, mx):
                    rows = pl.ds(al(c * CK, CK), CK)
                    s = jnp.dot(k_v[rows, :], w, preferred_element_type=F32)
                    sf_v[rows, :] = s
                    return fold(jnp.maximum, s, mx)
                mx = jax.lax.fori_loop(0, NC, p1, jnp.full((8, TQ), -jnp.inf, F32))
                m = jnp.max(mx, axis=0, keepdims=True)

                def p2(c, carry2):
                    acc, l = carry2
                    rows = pl.ds(al(c * CK, CK), CK)
                    p = jnp.exp2(sf_v[rows, :] - m)
                    o = jnp.dot(vt_v[:, rows], p.astype(BF16), preferred_element_type=F32)
                    return acc + o, fold(jnp.add, p, l)
                acc, l = jax.lax.fori_loop(
                    0, NC, p2, (jnp.zeros((DH, TQ), F32), jnp.zeros((8, TQ), F32)))
                put_ot(u, acc * (grow / jnp.sum(l, axis=0, keepdims=True)))
                return carry
            jax.lax.fori_loop(0, HPG, head, 0)

        def fix_up(tile):
            @pl.when(z_ref[1] != 0)
            def _():
                exact_attention(tile)

        def hidden(tile, half, f):
            xt = x_v[pl.ds(al(tile * TQ + half * TR, TR), TR), :]
            gb = jnp.broadcast_to(1.0 - g_v[tile * RH + half][0:1, :], (128, TR)).T
            gg = jnp.dot(xt, wg_v[f], preferred_element_type=F32)
            uu = jnp.dot(xt, wu_v[f], preferred_element_type=F32)
            hh = jnp.maximum(gg, 0.0) * uu
            return jnp.concatenate(
                [hh[:, j * 128:(j + 1) * 128] * gb for j in range(FC // 128)], axis=1).astype(BF16)

        def ffn_part(tile, t):
            f = t >> 1
            wo_g = wo_v[pl.ds(al(t * 128, 128), 128), :]

            def old(row):
                return jnp.where(t > 0, acc_v[pl.ds(row, TR), :], 0.0)

            half = t & 1
            row = al(tile * TQ + half * TR, TR)
            o_nat = ot_v[half].T.astype(BF16)
            hh = hidden(tile, half, f)
            y = jnp.dot(o_nat, wo_g, preferred_element_type=F32)
            y = y + jnp.dot(hh, wd_v[f], preferred_element_type=F32)
            y = y + old(row)
            acc_v[pl.ds(row, TR), :] = y
            o_v[pl.ds(row, TR), :] = y.astype(o_v.dtype)

            half1 = (t + 1) & 1
            row1 = al(tile * TQ + half1 * TR, TR)
            o_nat1 = ot_v[half1].T.astype(BF16)

            def tail():
                y1 = jnp.dot(o_nat1, wo_g, preferred_element_type=F32)
                acc_v[pl.ds(row1, TR), :] = y1 + old(row1)
            return tail

        z_ref[0] = 0
        z_ref[1] = 0
        for c_ in small_copies():
            c_.start()
        for c in range(RH):
            x_copy(c).start()
        wq_copy(0).start()
        for c in range(RH, XCH):
            x_copy(c).start()
        for t in BODY_SEM:
            for c_ in body_copies(t):
                c_.start()
        for c_ in small_copies():
            c_.wait()
        gw = gw_v[...].astype(F32)
        gw_row = jnp.concatenate([gw[r:r + 1, :] for r in range(D // 128)], axis=1)
        gw16 = jnp.broadcast_to(gw_row, (16, D)).astype(BF16)
        wkv_v[...] = jnp.concatenate([wvt_v[...], gw16, wkt_v[...]], axis=0)

        def kv_chunk(c):
            rows = pl.ds(al(c * TR, TR), TR)
            vt = jax.lax.dot_general(wkv_v[...], x_v[rows, :], NT, preferred_element_type=F32)
            ones = jnp.where(jax.lax.broadcasted_iota(I32, (16, TR), 0) < 2, 1.0, 0.0)
            ka = jnp.concatenate([vt[DH + 16:], ones], axis=0).T
            k_v[rows, :] = ka[:, 0:DH].astype(BF16)
            ka_v[rows, :] = ka.astype(BF16)
            vn_v[rows, :] = vt[:DH].T
            vt_v[:, rows] = vt[:DH].astype(BF16)
            g_v[c] = jax.nn.sigmoid(vt[DH:DH + 8])
            vb_v[c] = jnp.where(fold(jnp.maximum, jnp.abs(vt[:DH])) < 2.0 ** 60, 0.0, 1.0)

        def kb_rows(ds_):
            kf = k_v[0:NV, :].astype(F32)
            for d in ds_:
                kb_v[d] = jnp.broadcast_to(kf[:, d:d + 1], (NV, 128)).reshape(NV // 8, 8, 128)

        def vp_tile(c):
            rows_ = [vn_v[pl.ds(mk[c][0] + j * 16, 16), :] for j in range(mk[c][1] // 16 - 1, -1, -1)]
            if vk[c][1]:
                rows_ = [vn_v[pl.ds(*vk[c]), :]] + rows_
            vp_v[:, pl.ds(c * CK, CK)] = jnp.concatenate(rows_, axis=0).T.astype(BF16)

        def head_start(qh, dst):
            s = jnp.dot(k_v[0:NV, :], qh, preferred_element_type=F32)
            dst[...] = s
            return jnp.max(fold(jnp.maximum, s), axis=0, keepdims=True)

        for c in range(RH):
            x_copy(c).wait()
            kv_chunk(c)
        wq_copy(0).wait()
        qt0 = qproj_t(0, 0)
        mrows = [head_start(qt0[0:DH], p0_v)]
        mrows += [head_start(qt0[j * DH:(j + 1) * DH], sv_v.at[j - 1]) for j in range(1, HPG)]
        kb_rows(range(0, DH // 2))
        zv = jnp.full((8, TQ), z_ref[0], I32)
        for c in range(RH, 2 * RH):
            x_copy(c).wait()
        for c in range(RH, 2 * RH):
            kv_chunk(c)
        assert mk[PA - 1][0] + mk[PA - 1][1] <= 2 * TQ
        for c in range(PA):
            vp_tile(c)
        st0 = attention(qt0, mrows, 0, zv, tiles=list(range(PA)))
        qt1 = qproj_t(1, 0)
        m_new = head_start(qt1[0:DH], sv_v.at[HPG - 1])
        store_q(qt1, 0)
        kb_rows(range(DH // 2, DH))
        for c in range(2 * RH, XCH):
            x_copy(c).wait()
        for c in range(2 * RH, XCH):
            kv_chunk(c)
            if c == 3 * RH - 1:
                store_q(qproj_t(2, 0), 128)
                for b in range(LT):
                    for r in range(0, 128, 8):
                        spread_q(qa_v[b, DH + r:DH + r + 8, :], b, r)
        for c in range(PA, NC):
            vp_tile(c)
        z_ref[2] = jnp.max(vb_v[...]).astype(I32)
        attention(qt0, mrows, 0, zv, tiles=list(range(PA, NC)), st=st0)
        shift, m = shift_of(m_new)
        sh0_v[...] = shift
        p = jnp.exp2(sv_v[HPG - 1].reshape(NV // 8, 8, TQ) - m[None]).reshape(NV, TQ)
        l0_v[...] = fold(jnp.add, p)
        p0_v[...] = p

        def finish_tile(q):
            rows = pl.ds(q * TQ, TR)
            o_v[rows, :] = acc_v[rows, :].astype(o_v.dtype)
            out_copy(q).start()

        def body(it, carry):
            tile = it & (NQ - 1)
            t = it >> 2

            def rare(_, c0):
                for tt in BODY_SEM:
                    @pl.when(it == tt)
                    def _():
                        for c_ in body_copies(tt):
                            c_.wait()
                for q in range(NQ - 2):
                    @pl.when(it == NIT - NQ + 1 + q)
                    def _():
                        finish_tile(q)
                fix_up(tile)
                return c0
            is_rare = jnp.logical_or(
                jnp.logical_or(jnp.logical_or(it < 2, it > NIT - NQ), (it & (RH * NQ - 1)) == 0),
                z_ref[1] != 0)
            jax.lax.fori_loop(0, jnp.where(is_rare, 1, 0), rare, 0)

            zv = jnp.full((8, TQ), z_ref[0], I32)
            g3 = jnp.minimum(it + 3, NIT - 1)
            qt_new = qproj_t(g3 & (NQ - 1), g3 >> 2)
            mrows = [None] + vpu_chain(zv[:, :128])
            tail_fn = ffn_part(tile, t)
            qt = jnp.concatenate([qa_v[b, 0:128, :] for b in range(LT)], axis=1).astype(BF16)
            attention(qt, mrows, (it + 1) & (NQ - 1), zv, tail_fn, qt_new.astype(F32))
            for b in range(LT):
                qa_v[b, 0:128, :] = qa_v[b, 128:256, :]
            store_q(qt_new, 128)
            return carry
        jax.lax.fori_loop(0, NIT - 1, body, 0)
        finish_tile(NQ - 2)
        fix_up(NQ - 1)

        tile, t = NQ - 1, NG - 1
        half = t % RH
        other = 1 - half
        wo_g = wo_v[t * 128:(t + 1) * 128, :]
        hh = hidden(tile, half, t // RH)
        y = jnp.dot(ot_v[other].T.astype(BF16), wo_g, preferred_element_type=F32)
        rows = pl.ds(tile * TQ + other * TR, TR)
        o_v[rows, :] = (y + acc_v[rows, :]).astype(o_v.dtype)
        tail = [out_copy(tile, other * TR, TR)]
        o_nat = ot_v[half].T.astype(BF16)
        tail[0].start()
        ER = TR // ESPLIT
        for e in range(ESPLIT):
            lo = half * TR + e * ER
            y = jnp.dot(o_nat[e * ER:(e + 1) * ER], wo_g, preferred_element_type=F32)
            y = y + jnp.dot(hh[e * ER:(e + 1) * ER], wd_v[t // RH], preferred_element_type=F32)
            rows = pl.ds(tile * TQ + lo, ER)
            o_v[rows, :] = (y + acc_v[rows, :]).astype(o_v.dtype)
            tail.append(out_copy(tile, lo, ER, SEM_OUT + NQ + e))
            tail[-1].start()
        for q in range(NQ - 1):
            out_copy(q).wait()
        for c_ in tail:
            c_.wait()

    any_spec = pl.BlockSpec(memory_space=pl.ANY)
    out = pl.pallas_call(
        kernel,
        in_specs=[any_spec] * 9,
        out_specs=any_spec,
        out_shape=jax.ShapeDtypeStruct((S, D), A_x.dtype),
        scratch_shapes=[
            pltpu.VMEM((S, D), BF16),
            pltpu.VMEM((NG, D, 128), BF16),
            pltpu.VMEM((DH, D), BF16),
            pltpu.VMEM((DH, D), BF16),
            pltpu.VMEM((D, D), BF16),
            pltpu.VMEM((NF, D, FC), BF16),
            pltpu.VMEM((NF, D, FC), BF16),
            pltpu.VMEM((NF, FC, D), BF16),
            pltpu.VMEM((D // 128, 128), BF16),
            pltpu.VMEM((2 * DH + 16, D), BF16),
            pltpu.VMEM((S, DH), BF16),
            pltpu.VMEM((S, KA), BF16),
            pltpu.VMEM((DH, S), BF16),
            pltpu.VMEM((S, DH), F32),
            pltpu.VMEM((DH, S), BF16),
            pltpu.VMEM((XCH, 8, TR), F32),
            pltpu.VMEM((XCH, 8, TR), F32),
            pltpu.VMEM((DH, NV // 8, 8, 128), F32),
            pltpu.VMEM((LT, 256, 128), F32),
            pltpu.VMEM((LT, 128, 8, 128), F32),
            pltpu.VMEM((16, TQ), BF16),
            pltpu.VMEM((128, TQ), BF16),
            pltpu.VMEM((NV, TQ), F32),
            pltpu.VMEM((HPG, NV, TQ), F32),
            pltpu.VMEM((8, TQ), F32),
            pltpu.VMEM((RH, 128, TR), F32),
            pltpu.VMEM((S, D), F32),
            pltpu.VMEM((S, D), A_x.dtype),
            pltpu.VMEM((S, TQ), F32),
            pltpu.SMEM((3,), I32),
            pltpu.SemaphoreType.DMA((NSEM,)),
        ],
        compiler_params=pltpu.CompilerParams(vmem_limit_bytes=100 * 1024 * 1024),
        name="gated_mix",
    )(A_x.reshape(S, D), A_wq, A_wk.T, A_wv.T, A_wo, B_W_gate, B_W_up, B_W_down,
      gate_w.reshape(D // 128, 128))
    return out.reshape(1, S, D)
```
